```python
import os as _os
_os.environ.setdefault('JAX_PLATFORMS', 'cpu')
import jax
import jax.numpy as jnp

def _softmax(x, axis=-1):
    return jax.nn.softmax(x, axis=axis)

def _gelu(x):
    return jax.nn.gelu(x, approximate=True)

def _silu(x):
    return jax.nn.silu(x)

def _sigmoid(x):
    return jax.nn.sigmoid(x)

def _layernorm(x, axis=-1, eps=1e-05):
    m = jnp.mean(x, axis=axis, keepdims=True)
    v = jnp.var(x, axis=axis, keepdims=True)
    return (x - m) / jnp.sqrt(v + eps)

def _scatter_add(tgt, idx, src, axis=0):
    return tgt.at[idx].add(src)

def _segment_sum(src, seg, n):
    return jax.ops.segment_sum(src, seg, n)

class _Rng:

    def __init__(self, key):
        self._k = key

    def _next(self):
        self._k, sub = jax.random.split(self._k)
        return sub

    def normal(self, shape):
        return jax.random.normal(self._next(), shape, dtype=jnp.bfloat16)

    def randint(self, lo, hi, shape):
        return jax.random.randint(self._next(), shape, lo, hi, dtype=jnp.int32)

    def uniform(self, shape, lo=0.0, hi=1.0):
        return jax.random.uniform(self._next(), shape, jnp.bfloat16, lo, hi)

    def permutation(self, n):
        return jax.random.permutation(self._next(), n)
kernel_name = 'adaLN_cond__ssm_conv_h3__moe_arch_mod__prompt'

def setup_inputs():
    _rng = _Rng(jax.random.key(int.from_bytes(__import__("os").urandom(4), "little")))
    _w = lambda a: (lambda t: t.astype(jnp.bfloat16) if jnp.issubdtype(t.dtype, jnp.floating) else t)(jnp.asarray(a))

    def _A_setup():
        B, S, D = (1, 2048, 640)
        ks = 4
        return {'q': _w((lambda *s: _rng.normal(s) * 0.05)(B, S, D)), 'k': _w((lambda *s: _rng.normal(s) * 0.4)(B, S, D)), 'v': _w((lambda *s: _rng.normal(s) * 0.4)(B, S, D)), 'shift_k': _w((lambda *s: _rng.normal(s) * 0.4)(D, ks) * 0.5), 'ssm_k': _w((lambda *s: _rng.normal(s) * 0.4)(D, S) * (1.0 / S ** 0.5)), 'ssm_D': _w((lambda *s: _rng.normal(s) * 0.4)(D))}
    _A_in = _A_setup()

    def _B_setup():
        B, S, D, F, C = (1, 2048, 640, 1728, 2)
        return {'x': _w((lambda *s: _rng.normal(s) * 0.05)(B, S, D)), 'w_r': _w((lambda *s: _rng.normal(s) * 0.1)(D)), 'w_gate': _w((lambda *s: _rng.normal(s) * 0.1)(D, F)), 'w_up': _w((lambda *s: _rng.normal(s) * 0.1)(D, F)), 'w_down': _w((lambda *s: _rng.normal(s) * 0.1)(F, D))}
    _B_in = _B_setup()
    return {'A_q': _A_in['q'], 'A_k': _A_in['k'], 'A_v': _A_in['v'], 'A_shift_k': _A_in['shift_k'], 'A_ssm_k': _A_in['ssm_k'], 'A_ssm_D': _A_in['ssm_D'], 'B_x': _B_in['x'], 'B_w_r': _B_in['w_r'], 'B_w_gate': _B_in['w_gate'], 'B_w_up': _B_in['w_up'], 'B_w_down': _B_in['w_down'], 'c': _w((lambda *s: _rng.normal(s) * 0.2)(1, 640) * 8.0), 'w_mod': _w((lambda *s: _rng.normal(s) * 0.2)(640, 6 * 640) * 640 ** (-0.5) * 8.0)}

def reference(A_q, A_k, A_v, A_shift_k, A_ssm_k, A_ssm_D, B_x, B_w_r, B_w_gate, B_w_up, B_w_down, c, w_mod):

    def _A_ref(q, k, v, shift_k, ssm_k, ssm_D):
        B, S, D = q.shape
        ks = shift_k.shape[-1]
        k_pad = jnp.pad(k, ((0, 0), (ks - 1, 0), (0, 0)))
        k_shift = jnp.zeros_like(k)
        for t in range(ks):
            k_shift = k_shift + k_pad[:, t:t + S, :] * shift_k[:, ks - 1 - t][None, None, :]
        kv = k_shift * v
        L = 2 * S
        kv_pad = jnp.pad(kv, ((0, 0), (0, S), (0, 0)))
        kf_pad = jnp.pad(ssm_k, ((0, 0), (0, S)))
        kv_f = (lambda x, axes=(-2, -1): jnp.fft.rfft2(x.astype(jnp.float32), axes=axes))(kv_pad[:, None, :, :], axes=(1, 2))
        kf_f = (lambda x, axes=(-2, -1): jnp.fft.rfft2(x.astype(jnp.float32), axes=axes))(kf_pad[:, None, :], axes=(1, 2))
        kf_f = (lambda x, *d: x.transpose(*d))(kf_f, 1, 2, 0)
        y_f = kv_f * kf_f[None, :, :, :]
        y = (lambda x, s, axes=(-2, -1): jnp.fft.irfft2(x, s=s, axes=axes).astype(jnp.bfloat16))(y_f, (1, L), axes=(1, 2))[:, 0, :S, :]
        y = y + kv * ssm_D[None, None, :]
        return q * y

    def _B_ref(x, w_r, w_gate, w_up, w_down):
        B, S, D = x.shape
        C = 2
        r = x @ w_r
        idx = jnp.argsort(-r, axis=-1)[:, :C]
        idx_e = jnp.repeat(idx.reshape(B, C, 1), D, axis=2)
        x_sel = jnp.take_along_axis(x, idx_e, axis=1)
        g = _silu(x_sel @ w_gate)
        u = x_sel @ w_up
        y = g * u @ w_down
        r_sel = _sigmoid(jnp.take_along_axis(r, idx, axis=1))
        y = y * r_sel.reshape(B, C, 1)
        b_off = (jnp.arange(B) * S).reshape(B, 1)
        flat_idx = (idx + b_off).reshape(B * C)
        zero = (x * 0.0).reshape(B * S, D)
        upd = _scatter_add(zero, flat_idx, y.reshape(B * C, D), axis=0)
        return x + upd.reshape(B, S, D)
    x = A_q
    mod = (_silu(c) @ w_mod).reshape(c.shape[0], 6, 1, -1)
    sa, ca, ga, sb, cb, gb = (mod[:, 0].copy(), mod[:, 1].copy(), mod[:, 2].copy(), mod[:, 3].copy(), mod[:, 4].copy(), mod[:, 5].copy())
    h = _layernorm(x, axis=-1) * (1 + ca) + sa
    x = x + ga * _A_ref(h, A_k, A_v, A_shift_k, A_ssm_k, A_ssm_D)
    h = _layernorm(x, axis=-1) * (1 + cb) + sb
    x = x + gb * _B_ref(h, B_w_r, B_w_gate, B_w_up, B_w_down)
    return x
```

```python
import math

import jax
import jax.numpy as jnp
from jax import lax
import jax.experimental.pallas as pl
import jax.experimental.pallas.tpu as pltpu

S = 2048
D = 640
F = 1728
NJ = D // 128
NA = 4
NP = 4
EPS = 1e-5
OCH = 256
NOC = S // OCH

F32 = jnp.float32
BF16 = jnp.bfloat16
U32 = jnp.uint32

SEM_SK, SEM_DD, SEM_WR, SEM_C = 0, 1, 2, 3
SEM_SSM = 4
SEM_K = SEM_SSM + NJ
SEM_V = SEM_K + NJ
SEM_WM = SEM_V + NJ
SEM_Q = SEM_WM + 1
SEM_WG = SEM_Q + 2 * NJ
SEM_WU = SEM_WG + 1
SEM_WD = SEM_WU + 1
SEM_OUT = SEM_WD + 1
NSEM = SEM_OUT + NOC


def _lo(w):
    return lax.bitcast_convert_type(w << 16, F32)


def _hi(w):
    return lax.bitcast_convert_type(w & jnp.uint32(0xFFFF0000), F32)


def _cadd(x, y):
    return (x[0] + y[0], x[1] + y[1])


def _csub(x, y):
    return (x[0] - y[0], x[1] - y[1])


def _cadd_i(x, y):
    return (x[0] - y[1], x[1] + y[0])


def _csub_i(x, y):
    return (x[0] + y[1], x[1] - y[0])


def _cmul(x, y):
    return (x[0] * y[0] - x[1] * y[1], x[0] * y[1] + x[1] * y[0])


def _rb(x):
    return x.astype(BF16).astype(F32)


def _sum5(xs):
    return ((xs[0] + xs[1]) + (xs[2] + xs[3])) + xs[4]


def _ln_stats(xs):
    m = jnp.sum(_sum5(xs), axis=-1, keepdims=True) * (1.0 / D)
    xc = [x - m for x in xs]
    var = jnp.sum(_sum5([c * c for c in xc]), axis=-1, keepdims=True) * (1.0 / D)
    return xc, lax.rsqrt(var + EPS)


def _kernel(q_hbm, k_hbm, v_hbm, sk_hbm, ssm_hbm, dd_hbm, wr_hbm, wg_hbm, wu_hbm,
            wd_hbm, c_hbm, wm_hbm, out_hbm,
            kbuf, vbuf, qbuf, sbuf, wmbuf, wgbuf, wubuf, wdbuf,
            skbuf, ddbuf, wrbuf, cbuf,
            prm, gf, gi, ubuf, ktb, s1u, s1k, zbuf, ybuf, onat, obuf, rbuf, mp, sems):
    def cp(src, dst, s):
        return pltpu.make_async_copy(src, dst, sems.at[s])

    def lanes(j):
        if isinstance(j, int):
            return pl.ds(j * 128, 128)
        return pl.ds(pl.multiple_of(j * 128, 128), 128)

    def cp_ssm(j):
        return cp(ssm_hbm.at[lanes(j), :], sbuf.at[j], SEM_SSM + j)

    def cp_k(j):
        return cp(k_hbm.at[0, :, lanes(j)], kbuf.at[j, pl.ds(16, S), :], SEM_K + j)

    def cp_v(j):
        return cp(v_hbm.at[0, :, lanes(j)], vbuf.at[j], SEM_V + j)

    def cp_q(h, j):
        return cp(q_hbm.at[0, pl.ds(h * 1024, 1024), lanes(j)],
                  qbuf.at[j, pl.ds(h * 1024, 1024), :], SEM_Q + h * NJ + j)

    def cp_out(c):
        rows = pl.ds(c * OCH, OCH) if isinstance(c, int) else pl.ds(
            pl.multiple_of(c * OCH, OCH), OCH)
        return cp(obuf.at[rows, :], out_hbm.at[0, rows, :], SEM_OUT + c)

    cp_sk = cp(sk_hbm, skbuf, SEM_SK)
    cp_dd = cp(dd_hbm, ddbuf, SEM_DD)
    cp_wr = cp(wr_hbm, wrbuf, SEM_WR)
    cp_c = cp(c_hbm, cbuf, SEM_C)
    cp_wm = cp(wm_hbm, wmbuf, SEM_WM)
    cp_wg = cp(wg_hbm, wgbuf, SEM_WG)
    cp_wu = cp(wu_hbm, wubuf, SEM_WU)
    cp_wd = cp(wd_hbm, wdbuf, SEM_WD)

    for j in range(NJ):
        kbuf[j, pl.ds(0, 16), :] = jnp.zeros((16, 128), BF16)

    cp_ssm(0).start()
    cp_k(0).start()
    cp_v(0).start()
    cp_sk.start()
    cp_dd.start()
    cp_wr.start()
    cp_c.start()
    for j in range(1, NJ):
        cp_ssm(j).start()
        cp_k(j).start()
        cp_v(j).start()
    cp_wm.start()
    for h in range(2):
        for j in range(NJ):
            cp_q(h, j).start()
    cp_wg.start()
    cp_wu.start()
    cp_wd.start()

    rho = lax.broadcasted_iota(jnp.int32, (256, 128), 0)
    col = lax.broadcasted_iota(jnp.int32, (256, 128), 1)
    n8 = ((rho >> 4) << 3) + (rho & 7)
    f1 = jnp.where(n8 < 64, 2 * n8, 2 * n8 - 127)
    quad = ((rho >> 3) & 1) * 512
    for p in range(NP):
        n = ((2 * f1 + 1) * (4 * col + p) + quad) & 2047
        g = jnp.cos(n.astype(F32) * (math.pi / 1024.0))
        gf[p] = g.astype(BF16)
        gi[p] = (g.T * (2.0 / 1024.0)).astype(BF16)

    cp_sk.wait()
    cp_dd.wait()
    skf = skbuf[...].astype(F32)
    ddf = ddbuf[...].astype(F32).reshape(1, D)
    for j in range(NJ):
        prm[j, pl.ds(0, 4), :] = skf[:, j * 128:(j + 1) * 128]
        prm[j, pl.ds(4, 1), :] = ddf[:, j * 128:(j + 1) * 128]

    k32 = kbuf.bitcast(U32)
    v32 = vbuf.bitcast(U32)
    q32 = qbuf.bitcast(U32)

    def vpu_group(j, g, dvec):
        plus = g < 8
        re = pl.ds(16 * g, 8)
        im = pl.ds(16 * g + 8, 8)

        def ld(ref, a, p):
            return (ref[4 * a + p, re, :], ref[4 * a + p, im, :])

        def ldk(a, p):
            x = ld(s1k, a, p)
            if a == 0 and p == 0:
                x = (x[0] + dvec, x[1])
            return x

        def half(odd):
            us, ks = [], []
            for a in range(NA):
                for (lst, get) in ((us, lambda p: ld(s1u, a, p)), (ks, lambda p: ldk(a, p))):
                    if not odd:
                        e0 = _cadd(get(0), get(2))
                        e1 = _cadd(get(1), get(3))
                        lst.append((_cadd(e0, e1), _csub(e0, e1)))
                    else:
                        e0 = _csub(get(0), get(2))
                        e1 = _csub(get(1), get(3))
                        lst.append((_csub_i(e0, e1), _cadd_i(e0, e1)))
            outs = [[None, None] for _ in range(NA)]
            for f in range(2):
                kt = [ks[0][f]]
                for a in range(1, NA):
                    kt.append(_cadd_i(ks[a][f], ks[a - 1][f]) if plus
                              else _csub_i(ks[a][f], ks[a - 1][f]))
                for a in range(NA):
                    acc = _cmul(us[a][f], kt[0])
                    for jj in range(1, a + 1):
                        acc = _cadd(acc, _cmul(us[a - jj][f], kt[jj]))
                    outs[a][f] = acc
            return [(_cadd(o[0], o[1]), _csub(o[0], o[1])) for o in outs]

        ev = half(False)
        od = half(True)
        rows = pl.ds(16 * g, 16)
        for a in range(NA):
            z = (_cadd(ev[a][0], od[a][0]), _cadd_i(ev[a][1], od[a][1]),
                 _csub(ev[a][0], od[a][0]), _csub_i(ev[a][1], od[a][1]))
            for p in range(NP):
                zbuf[j, 4 * a + p, rows, :] = jnp.concatenate(z[p], axis=0).astype(BF16)

    def phase_a(j, carry):
        cp_ssm(j).wait()
        for a in range(NA):
            kt = sbuf[j, :, pl.ds(512 * a, 512)].astype(F32).T
            ktb[pl.ds(512 * a, 512), :] = kt
        for a in range(NA):
            for p in range(NP):
                kp = ktb[pl.ds(512 * a + p, 128, stride=4), :].astype(BF16)
                s1k[4 * a + p] = jnp.dot(gf[p], kp, preferred_element_type=F32)
        cp_k(j).wait()
        cp_v(j).wait()
        taps = [prm[j, pl.ds(m, 1), :] for m in range(4)]
        dvec = prm[j, pl.ds(4, 1), :]
        for a in range(NA):
            for rb in range(8):
                base = 256 * a + 32 * rb
                w0 = k32[j, pl.ds(8 + base, 16, stride=2), :]
                w1 = k32[j, pl.ds(8 + base + 1, 16, stride=2), :]
                p0 = k32[j, pl.ds(8 + base - 2, 16, stride=2), :]
                p1 = k32[j, pl.ds(8 + base - 1, 16, stride=2), :]
                x0 = v32[j, pl.ds(base, 16, stride=2), :]
                x1 = v32[j, pl.ds(base + 1, 16, stride=2), :]
                seq = [_hi(p0), _lo(p1), _hi(p1), _lo(w0), _hi(w0), _lo(w1), _hi(w1)]
                vv = [_lo(x0), _hi(x0), _lo(x1), _hi(x1)]
                for p in range(NP):
                    ks = ((seq[p] * taps[3] + seq[p + 1] * taps[2])
                          + (seq[p + 2] * taps[1] + seq[p + 3] * taps[0]))
                    ubuf[4 * a + p, pl.ds(16 * rb, 16), :] = (ks * vv[p]).astype(BF16)
            for p in range(NP):
                s1u[4 * a + p] = jnp.dot(gf[p], ubuf[4 * a + p], preferred_element_type=F32)
        for g in range(16):
            vpu_group(j, g, dvec)
        return carry

    lax.fori_loop(0, NJ, phase_a, 0)

    cp_c.wait()
    cp_wr.wait()
    cp_wm.wait()
    cf = cbuf[...].astype(F32)
    sc = (cf * jax.nn.sigmoid(cf)).astype(BF16)
    mod = jnp.dot(jnp.broadcast_to(sc, (16, D)), wmbuf[...],
                  preferred_element_type=F32)[0:1, :]
    mod = _rb(mod)
    sa, ca, ga, sb, cb, gb = [mod[:, i * D:(i + 1) * D] for i in range(6)]
    ca1 = _rb(1.0 + ca)
    cb1 = _rb(1.0 + cb)
    wrf = wrbuf[...].astype(F32).reshape(1, D)
    r0 = jnp.sum(wrf * sb, axis=-1, keepdims=True)
    mp[pl.ds(0, 1), :] = ga * ca1
    mp[pl.ds(1, 1), :] = ga * sa
    mp[pl.ds(2, 1), :] = gb * cb1
    mp[pl.ds(3, 1), :] = gb * sb
    mp[pl.ds(4, 1), :] = wrf * cb1
    mp[pl.ds(5, 1), :] = cb1
    mp[pl.ds(6, 1), :] = sb
    mp[pl.ds(7, 1), :] = gb

    def mrow(r):
        return [mp[pl.ds(r, 1), pl.ds(j * 128, 128)] for j in range(NJ)]

    def mix(xs, ys):
        a1, a0 = mrow(0), mrow(1)
        xc, rs = _ln_stats(xs)
        x1 = [xs[j] + ((xc[j] * rs) * a1[j] + a0[j]) * ys[j] for j in range(NJ)]
        xc2, rs2 = _ln_stats(x1)
        return x1, [c * rs2 for c in xc2]

    def phase_b(a, s):
        for pp in range(2):
            p = 2 * s + pp
            for j in range(NJ):
                ybuf[4 * a + p, j] = jnp.dot(gi[p], zbuf[j, 4 * a + p],
                                             preferred_element_type=F32)
        b1, b0, w1 = mrow(2), mrow(3), mrow(4)
        for rg in range(16):
            words = [q32[j, pl.ds(256 * a + s + 16 * rg, 8, stride=2), :] for j in range(NJ)]
            for pp in range(2):
                p = 2 * s + pp
                xs = [(_hi if pp else _lo)(w) for w in words]
                ys = [ybuf[4 * a + p, j, pl.ds(8 * rg, 8), :] for j in range(NJ)]
                x1, n2 = mix(xs, ys)
                r = jnp.sum(_sum5([n2[j] * w1[j] for j in range(NJ)]), axis=-1,
                            keepdims=True)
                rbuf[pl.ds(8 * rg, 8), pl.ds(4 * a + p, 1)] = r
                for j in range(NJ):
                    onat[j, pl.ds(512 * a + 32 * rg + p, 8, stride=4), :] = (
                        x1[j] + (n2[j] * b1[j] + b0[j]))

    for a in range(NA):
        if a % 2 == 0:
            for j in range(NJ):
                cp_q(a // 2, j).wait()
        for s in range(2):
            phase_b(a, s)
        for j in range(NJ):
            obuf[pl.ds(512 * a, 512), pl.ds(j * 128, 128)] = (
                onat[j, pl.ds(512 * a, 512), :].astype(BF16))

    rr = _rb(rbuf[...] + r0)
    ri = lax.broadcasted_iota(jnp.int32, (128, 16), 0)
    ci = lax.broadcasted_iota(jnp.int32, (128, 16), 1)
    tok = (ci >> 2) * 512 + ri * 4 + (ci & 3)
    m1 = jnp.max(rr)
    t1 = jnp.minimum(jnp.min(jnp.where(rr == m1, tok, S)), S - 1)
    rr2 = jnp.where(tok == t1, -jnp.inf, rr)
    m2 = jnp.max(rr2)
    t2 = jnp.min(jnp.where(jnp.logical_and(rr2 == m2, tok != t1), tok, S))
    t2 = jnp.where(t2 >= S, jnp.where(t1 == 0, 1, 0), t2)
    c1 = t1 // OCH
    c2 = t2 // OCH

    first = lax.broadcasted_iota(jnp.int32, (16, 128), 0) == 0

    def pick(get):
        return [jnp.where(first, jnp.broadcast_to(get(t1, j), (16, 128)),
                          jnp.broadcast_to(get(t2, j), (16, 128))) for j in range(NJ)]

    def get_q(t, j):
        w = q32[j, pl.ds(t >> 1, 1), :]
        return jnp.where((t & 1) == 1, _hi(w), _lo(w))

    def get_y(t, j):
        return ybuf[((t >> 9) << 2) + (t & 3), j, pl.ds((t >> 2) & 127, 1), :]

    x1s, n2s = mix(pick(get_q), pick(get_y))
    cb1r, sbr, gbr = mrow(5), mrow(6), mrow(7)
    h2 = [n2s[j] * cb1r[j] + sbr[j] for j in range(NJ)]
    hb = jnp.concatenate(h2, axis=1).astype(BF16)
    nt = (((1,), (1,)), ((), ()))
    cp_wg.wait()
    gg = lax.dot_general(hb, wgbuf[...], nt, preferred_element_type=F32)
    cp_wu.wait()
    uu = lax.dot_general(hb, wubuf[...], nt, preferred_element_type=F32)
    act = (gg * jax.nn.sigmoid(gg) * uu).astype(BF16)
    cp_wd.wait()
    for c in range(NOC):
        @pl.when(jnp.logical_and(c1 != c, c2 != c))
        def _():
            cp_out(c).start()
    yy = jnp.dot(act, wdbuf[...], preferred_element_type=F32)
    rsel = jnp.where(first[:, 0:1], m1, m2)
    yy = yy * jax.nn.sigmoid(rsel)
    new = jnp.concatenate(
        [x1s[j] + gbr[j] * (h2[j] + yy[:, j * 128:(j + 1) * 128]) for j in range(NJ)],
        axis=1)
    rowi = lax.broadcasted_iota(jnp.int32, (16, D), 0)
    for (t, r) in ((t1, 0), (t2, 1)):
        blk = pl.ds(pl.multiple_of((t >> 4) << 4, 16), 16)
        old = obuf[blk, :].astype(F32)
        obuf[blk, :] = jnp.where(rowi == (t & 15),
                                 jnp.broadcast_to(new[r:r + 1, :], (16, D)),
                                 old).astype(BF16)
    cp_out(c1).start()

    @pl.when(c2 != c1)
    def _():
        cp_out(c2).start()

    for c in range(NOC):
        cp_out(c).wait()


@jax.jit
def pallas_adaLN_cond__ssm_conv_h3__moe_arch_mod__prompt_kernel(
    A_q: jax.Array,
    A_k: jax.Array,
    A_v: jax.Array,
    A_shift_k: jax.Array,
    A_ssm_k: jax.Array,
    A_ssm_D: jax.Array,
    B_x: jax.Array,
    B_w_r: jax.Array,
    B_w_gate: jax.Array,
    B_w_up: jax.Array,
    B_w_down: jax.Array,
    c: jax.Array,
    w_mod: jax.Array,
):
    del B_x
    args = (A_q, A_k, A_v, A_shift_k.T, A_ssm_k, A_ssm_D, B_w_r, B_w_gate.T,
            B_w_up.T, B_w_down, c, w_mod)
    V = pltpu.VMEM
    scratch = [
        V((NJ, S + 16, 128), BF16),
        V((NJ, S, 128), BF16),
        V((NJ, S, 128), BF16),
        V((NJ, 128, S), BF16),
        V((D, 6 * D), BF16),
        V((F, D), BF16),
        V((F, D), BF16),
        V((F, D), BF16),
        V((4, D), BF16),
        V((D,), BF16),
        V((D,), BF16),
        V((1, D), BF16),
        V((NJ, 8, 128), F32),
        V((NP, 256, 128), BF16),
        V((NP, 128, 256), BF16),
        V((16, 128, 128), BF16),
        V((S, 128), F32),
        V((16, 256, 128), F32),
        V((16, 256, 128), F32),
        V((NJ, 16, 256, 128), BF16),
        V((16, NJ, 128, 128), F32),
        V((NJ, S, 128), F32),
        V((S, D), BF16),
        V((128, 16), F32),
        V((8, D), F32),
        pltpu.SemaphoreType.DMA((NSEM,)),
    ]
    return pl.pallas_call(
        _kernel,
        out_shape=jax.ShapeDtypeStruct((1, S, D), BF16),
        in_specs=[pl.BlockSpec(memory_space=pl.ANY)] * len(args),
        out_specs=pl.BlockSpec(memory_space=pl.ANY),
        scratch_shapes=scratch,
        compiler_params=pltpu.CompilerParams(vmem_limit_bytes=100 * 1024 * 1024),
    )(*args)
```

```python
import math

import jax
import jax.numpy as jnp
from jax import lax
import jax.experimental.pallas as pl
import jax.experimental.pallas.tpu as pltpu

S = 2048
D = 640
F = 1728
NJ = D // 128
NA = 4
NP = 4
EPS = 1e-5
FL = S * NJ
OCH = 8
EB = 8
QSPLIT = 128 // EB + 3

F32 = jnp.float32
BF16 = jnp.bfloat16
U32 = jnp.uint32
I32 = jnp.int32

SEM_SK, SEM_DD, SEM_WR, SEM_C = 0, 1, 2, 3
SEM_SSM = 4
SEM_K = SEM_SSM + NJ
SEM_V = SEM_K + NA
SEM_WM = SEM_V + NA
SEM_Q = SEM_WM + 1
SEM_WG = SEM_Q + 2
SEM_WU = SEM_WG + 1
SEM_WD = SEM_WU + 1
SEM_OUT = SEM_WD + 1
NSEM = SEM_OUT + OCH


def _lo(w):
    return lax.bitcast_convert_type(w << 16, F32)


def _hi(w):
    return lax.bitcast_convert_type(w & jnp.uint32(0xFFFF0000), F32)


def _pack(x):
    return pltpu.bitcast(x.astype(BF16), U32)


def _unpack(w):
    return pltpu.bitcast(w, BF16)


def _cadd(x, y):
    return (x[0] + y[0], x[1] + y[1])


def _csub(x, y):
    return (x[0] - y[0], x[1] - y[1])


def _cadd_i(x, y):
    return (x[0] - y[1], x[1] + y[0])


def _csub_i(x, y):
    return (x[0] + y[1], x[1] - y[0])


def _cmul(x, y):
    return (x[0] * y[0] - x[1] * y[1], x[0] * y[1] + x[1] * y[0])


def _rb(x):
    return x.astype(BF16).astype(F32)


def _sum5(xs):
    return ((xs[0] + xs[1]) + (xs[2] + xs[3])) + xs[4]


def _ln_stats(xs):
    m = jnp.sum(_sum5(xs), axis=-1, keepdims=True) * (1.0 / D)
    xc = [x - m for x in xs]
    var = jnp.sum(_sum5([c * c for c in xc]), axis=-1, keepdims=True) * (1.0 / D)
    return xc, lax.rsqrt(var + EPS)


def _cos_table(n):
    z = (jnp.abs(n - 1024) - 512).astype(F32) * (math.pi / 1024.0)
    z2 = z * z
    acc = jnp.full(z.shape, -1.0 / 39916800.0, F32)
    for cf in (1.0 / 362880.0, -1.0 / 5040.0, 1.0 / 120.0, -1.0 / 6.0, 1.0):
        acc = acc * z2 + cf
    return acc * z


def _mo(x, m):
    return x if isinstance(x, int) else pl.multiple_of(x, m)


def _kernel(q_hbm, k_hbm, v_hbm, sk_hbm, ssm_hbm, dd_hbm, wr_hbm, wg_hbm, wu_hbm,
            wd_hbm, c_hbm, wm_hbm, out_hbm,
            kbuf, vbuf, qbuf, sbuf, wmbuf, wgbuf, wubuf, wdbuf,
            skbuf, ddbuf, wrbuf, cbuf,
            prm, gfu, gfk, gi, ktb, s1u, s1k, kraw, za, zb_, ybuf, xcb, x1b, xc2b, st0, st1_, st2_, st3_, obuf, mp, sems):
    st = (st0, st1_, st2_, st3_)
    def cp(src, dst, s):
        return pltpu.make_async_copy(src, dst, sems.at[s])

    CR = FL // NA

    def cp_ssm(j):
        return cp(ssm_hbm.at[pl.ds(_mo(j * 128, 128), 128), :], sbuf.at[j], SEM_SSM + j)

    def cp_k(a):
        return cp(k_hbm.at[pl.ds(_mo(a * CR, 8), CR), :],
                  kbuf.at[pl.ds(_mo(40 + a * CR, 8), CR), :], SEM_K + a)

    def cp_v(a):
        rows = pl.ds(_mo(a * CR, 8), CR)
        return cp(v_hbm.at[rows, :], vbuf.at[rows, :], SEM_V + a)

    def cp_q(h):
        cut = QSPLIT * EB * 40
        rows = pl.ds(0, cut) if h == 0 else pl.ds(cut, FL - cut)
        return cp(q_hbm.at[rows, :], qbuf.at[rows, :], SEM_Q + h)

    def cp_out(c):
        rows = pl.ds(_mo(c * (FL // OCH), 8), FL // OCH)
        return cp(obuf.at[rows, :], out_hbm.at[rows, :], SEM_OUT + c)

    cp_sk = cp(sk_hbm, skbuf, SEM_SK)
    cp_dd = cp(dd_hbm, ddbuf, SEM_DD)
    cp_wr = cp(wr_hbm, wrbuf, SEM_WR)
    cp_c = cp(c_hbm, cbuf, SEM_C)
    cp_wm = cp(wm_hbm, wmbuf, SEM_WM)
    cp_wg = cp(wg_hbm, wgbuf, SEM_WG)
    cp_wu = cp(wu_hbm, wubuf, SEM_WU)
    cp_wd = cp(wd_hbm, wdbuf, SEM_WD)

    for j in range(NJ):
        cp_ssm(j).start()
    cp_sk.start()
    cp_dd.start()
    cp_wr.start()
    cp_c.start()
    for a in range(NA):
        cp_k(a).start()
        cp_v(a).start()
    cp_wm.start()
    cp_q(0).start()
    cp_q(1).start()
    cp_wg.start()
    cp_wu.start()
    cp_wd.start()

    k32 = kbuf.bitcast(U32)
    v32 = vbuf.bitcast(U32)
    q32 = qbuf.bitcast(U32)
    o32 = obuf.bitcast(U32)
    kbuf[pl.ds(0, 40), :] = jnp.zeros((40, 128), BF16)

    for hb in range(2):
        rho = lax.broadcasted_iota(I32, (128, 128), 0) + 128 * hb
        col = lax.broadcasted_iota(I32, (128, 128), 1)
        n8 = ((rho >> 4) << 3) + (rho & 7)
        odd = 4 * n8 + (1 if hb == 0 else -253)
        quad = ((rho >> 3) & 1) * 512
        iu = ((col >> 4) << 4) + ((col & 7) << 1) + ((col >> 3) & 1)
        nk = odd * (4 * col) + quad
        nu = odd * (4 * iu) + quad
        for p in range(NP):
            tk = _cos_table((nk + p * odd) & 2047)
            gfk[p, pl.ds(128 * hb, 128), :] = tk.astype(BF16)
            gi[p, hb] = (tk.T * (2.0 / 1024.0)).astype(BF16)
            gfu[p, pl.ds(128 * hb, 128), :] = _cos_table((nu + p * odd) & 2047).astype(BF16)
    gfk32 = gfk.bitcast(U32)
    gfu32 = gfu.bitcast(U32)
    gi32 = gi.bitcast(U32)

    cp_sk.wait()
    cp_dd.wait()
    skf = skbuf[...].astype(F32)
    ddf = ddbuf[...].astype(F32).reshape(1, D)
    for j in range(NJ):
        for m in range(4):
            prm[j, m] = jnp.broadcast_to(skf[m:m + 1, j * 128:(j + 1) * 128], (8, 128))
        prm[j, 4] = jnp.broadcast_to(ddf[:, j * 128:(j + 1) * 128], (8, 128))

    def fft4(ys, g):
        x = [(y[16 * g:16 * g + 8, :], y[16 * g + 8:16 * g + 16, :]) for y in ys]
        e0, e1 = _cadd(x[0], x[2]), _cadd(x[1], x[3])
        d0, d1 = _csub(x[0], x[2]), _csub(x[1], x[3])
        return (_cadd(e0, e1), _csub_i(d0, d1), _csub(e0, e1), _cadd_i(d0, d1))

    def cst(ref, idx, g, val):
        ref[idx + (pl.ds(16 * g, 8), slice(None))] = val[0]
        ref[idx + (pl.ds(16 * g + 8, 8), slice(None))] = val[1]

    def cld(ref, idx, g):
        return (ref[idx + (pl.ds(16 * g, 8), slice(None))],
                ref[idx + (pl.ds(16 * g + 8, 8), slice(None))])

    def fft4_store(dst, j, a, ys):
        for g in range(16):
            outs = fft4(ys, g)
            for f in range(4):
                cst(dst, (j, 4 * a + f), g, outs[f])

    def fwd_k(j, carry):
        cp_ssm(j).wait()
        for a in range(NA):
            ktb[pl.ds(512 * a, 512), :] = sbuf[j, :, pl.ds(512 * a, 512)].astype(F32).T
            ys = []
            for p in range(NP):
                kp = ktb[pl.ds(512 * a + p, 128, stride=4), :].astype(BF16)
                ys.append(jnp.dot(_unpack(gfk32[p]), kp, preferred_element_type=F32))
            for g in range(16):
                outs = fft4(ys, g)
                for f in range(4):
                    val = outs[f]
                    if a == 0:
                        val = (val[0] + prm[j, 4], val[1])
                    if 0 < a < NA - 1:
                        cst(kraw, (a - 1, f), g, val)
                    if a > 0:
                        prev = cld(s1k, (j, f), g) if a == 1 else cld(kraw, (a - 2, f), g)
                        val = _cadd_i(val, prev) if g < 8 else _csub_i(val, prev)
                    cst(s1k, (j, 4 * a + f), g, val)
        return carry

    lax.fori_loop(0, NJ, fwd_k, 0)

    def fwd_u(a, carry):
        cp_k(a).wait()
        cp_v(a).wait()
        kc = k32.at[pl.ds(_mo(a * 1280, 8), 1304)]
        vc = v32.at[pl.ds(_mo(a * 1280, 8), 1280)]
        for j in range(NJ):
            ub = [[] for _ in range(NP)]
            for b in range(8):
                base = b * 160 + 4 * j
                kw = [kc[pl.ds(base + 20 + w, 8, stride=20), :] for w in range(4)]
                pw = [kc[pl.ds(base + w, 8, stride=20), :] for w in (2, 3)]
                vw = [vc[pl.ds(base + w, 8, stride=20), :] for w in range(4)]
                seq = [_hi(pw[0]), _lo(pw[1]), _hi(pw[1])]
                vv = []
                for w in range(4):
                    seq += [_lo(kw[w]), _hi(kw[w])]
                    vv += [_lo(vw[w]), _hi(vw[w])]
                for ph in range(8):
                    ks = ((seq[ph] * prm[j, 3] + seq[ph + 1] * prm[j, 2])
                          + (seq[ph + 2] * prm[j, 1] + seq[ph + 3] * prm[j, 0]))
                    ub[ph % 4].append(ks * vv[ph])
            ys = [jnp.dot(_unpack(gfu32[p]), jnp.concatenate(ub[p], axis=0).astype(BF16),
                          preferred_element_type=F32) for p in range(NP)]
            fft4_store(s1u, j, a, ys)
        return carry

    lax.fori_loop(0, NA, fwd_u, 0)

    def vpu_group(j, zb, g):
        for a in range(NA):
            zf = []
            for f in range(4):
                acc = None
                for jj in range(a + 1):
                    t = _cmul(cld(s1u, (j, 4 * (a - jj) + f), g), cld(s1k, (j, 4 * jj + f), g))
                    acc = t if acc is None else _cadd(acc, t)
                zf.append(acc)
            e0, e1 = _cadd(zf[0], zf[2]), _csub(zf[0], zf[2])
            o0, o1 = _cadd(zf[1], zf[3]), _csub(zf[1], zf[3])
            z = (_cadd(e0, o0), _cadd_i(e1, o1), _csub(e0, o0), _csub_i(e1, o1))
            for p in range(NP):
                cst(zb, (4 * a + p,), g, z[p])

    def inv_unit(j, zb, n):
        a, p = n // NP, n % NP
        lhs = jnp.concatenate([_unpack(gi32[p, 0]), _unpack(gi32[p, 1])], axis=1)
        ybuf[j, pl.ds(512 * a + p, 128, stride=4), :] = jnp.dot(
            lhs, zb[n].astype(BF16), preferred_element_type=F32)

    for g in range(16):
        vpu_group(0, za, g)

    def v_step(i, carry):
        j = 2 * i + 1
        for g in range(16):
            inv_unit(j - 1, za, g)
            vpu_group(j, zb_, g)
        for g in range(16):
            inv_unit(j, zb_, g)
            vpu_group(j + 1, za, g)
        return carry

    lax.fori_loop(0, 2, v_step, 0)

    cp_c.wait()
    cp_wr.wait()
    cp_wm.wait()
    cp_q(0).wait()
    for n in range(16):
        inv_unit(NJ - 1, za, n)
    cf = cbuf[...].astype(F32)
    sc = (cf * jax.nn.sigmoid(cf)).astype(BF16)
    mod = jnp.dot(jnp.broadcast_to(sc, (16, D)), wmbuf[...],
                  preferred_element_type=F32)[0:8, :]
    mod = _rb(mod)
    sa, ca, ga, sb, cb, gb = [mod[:, i * D:(i + 1) * D] for i in range(6)]
    ca1 = _rb(1.0 + ca)
    cb1 = _rb(1.0 + cb)
    wrf = jnp.broadcast_to(wrbuf[...].astype(F32).reshape(1, D), (8, D))
    r0 = jnp.sum(wrf * sb, axis=-1, keepdims=True)
    sqd = math.sqrt(D)
    for i, val in enumerate((ga * ca1 * sqd, ga * sa, gb * cb1 * sqd, gb * sb,
                             wrf * cb1 * sqd, cb1 * sqd, sb, gb)):
        mp[i] = val

    def mrow(i):
        return [mp[i, :, pl.ds(j * 128, 128)] for j in range(NJ)]

    lane = lax.broadcasted_iota(I32, (8, 128), 1)

    def rsum(xs):
        return jnp.broadcast_to(jnp.sum(_sum5(xs), axis=-1, keepdims=True), (8, 128))

    def qtiles(blk):
        xs = []
        for m in range(EB // 2):
            xq = _unpack(q32[pl.ds(_mo((blk * (EB // 2) + m) * 40, 8), 40), :]).astype(F32)
            for h in range(2):
                xs.append([xq[40 * h + 8 * j:40 * h + 8 * j + 8, :] for j in range(NJ)])
        return xs

    def trows(blk, i):
        return pl.ds(_mo((blk * EB + i) * 8, 8), 8)

    def st1(blk, racc):
        for i, xs in enumerate(qtiles(blk)):
            st[0][blk * EB + i] = rsum(xs) * (1.0 / D)
        return racc

    def st2(blk, racc):
        for i, xs in enumerate(qtiles(blk)):
            m1 = st[0][blk * EB + i]
            xc = [x - m1 for x in xs]
            for j in range(NJ):
                xcb[j, trows(blk, i), :] = xc[j]
            st[1][blk * EB + i] = lax.rsqrt(rsum([c * c for c in xc]) + D * EPS)
        return racc

    def st3(blk, racc):
        a1, a0 = mrow(0), mrow(1)
        for i in range(EB):
            rs = st[1][blk * EB + i]
            x1 = []
            for j in range(NJ):
                xc = xcb[j, trows(blk, i), :]
                x1.append(xc + ((xc * rs) * a1[j] + a0[j]) * ybuf[j, trows(blk, i), :])
                x1b[j, trows(blk, i), :] = x1[j]
            st[2][blk * EB + i] = rsum(x1) * (1.0 / D)
        return racc

    def st4(blk, racc):
        w1 = mrow(4)
        for i in range(EB):
            m2 = st[2][blk * EB + i]
            xc = [x1b[j, trows(blk, i), :] - m2 for j in range(NJ)]
            for j in range(NJ):
                xc2b[j, trows(blk, i), :] = xc[j]
            rs = lax.rsqrt(rsum([c * c for c in xc]) + D * EPS)
            st[3][blk * EB + i] = rs
            r = rsum([xc[j] * w1[j] for j in range(NJ)]) * rs
            racc = jnp.where(lane == ((blk * EB + i) & 127), r, racc)
        return racc

    def st5(blk, racc):
        b1, b0 = mrow(2), mrow(3)
        for m in range(EB // 2):
            outs = []
            for h in range(2):
                i = 2 * m + h
                rs = st[3][blk * EB + i]
                mm = st[0][blk * EB + i] + st[2][blk * EB + i]
                outs += [xc2b[j, trows(blk, i), :] * (rs * b1[j] + 1.0) + (b0[j] + mm)
                         for j in range(NJ)]
            obuf[pl.ds(_mo((blk * (EB // 2) + m) * 80, 16), 80), :] = (
                jnp.concatenate(outs, axis=0).astype(BF16))
        return racc

    stages = (st1, st2, st3, st4, st5)
    NB = 256 // EB

    def epi(n, racc):
        for k, fn in reversed(list(enumerate(stages))):
            if isinstance(n, int) and not 0 <= n - k < NB:
                continue
            racc = fn(n - k, racc)
        return racc

    ra = jnp.zeros((8, 128), F32)
    for n in range(4):
        ra = epi(n, ra)
    ra = lax.fori_loop(4, QSPLIT, epi, ra)
    cp_q(1).wait()
    rb_ = lax.fori_loop(QSPLIT, NB, epi, jnp.zeros((8, 128), F32))
    for n in range(NB, NB + 4):
        rb_ = epi(n, rb_)

    rr = _rb(jnp.concatenate([ra, rb_], axis=1) + r0)
    tok = (lax.broadcasted_iota(I32, (8, 256), 1) * 8
           + lax.broadcasted_iota(I32, (8, 256), 0))

    def amax(x):
        return jnp.max(jnp.max(x, axis=1, keepdims=True), axis=0, keepdims=True)

    def amin(x):
        return jnp.min(jnp.min(x, axis=1, keepdims=True), axis=0, keepdims=True)

    m1 = amax(rr)
    t1v = jnp.minimum(amin(jnp.where(rr == m1, tok, S)), S - 1)
    rr2 = jnp.where(tok == t1v, -jnp.inf, rr)
    m2 = amax(rr2)
    t2v = amin(jnp.where(jnp.logical_and(rr2 == m2, tok != t1v), tok, S))
    t2v = jnp.where(t2v >= S, jnp.where(t1v == 0, 1, 0), t2v)
    t1 = t1v[0, 0]
    t2 = t2v[0, 0]
    c1 = t1 // (S // OCH)
    c2 = t2 // (S // OCH)

    first = lax.broadcasted_iota(I32, (8, 128), 0) == 0

    def pick(get):
        return [jnp.where(first, jnp.broadcast_to(get(t1, j), (8, 128)),
                          jnp.broadcast_to(get(t2, j), (8, 128))) for j in range(NJ)]

    def wrow(t, j):
        return pl.ds((t >> 3) * 20 + 4 * j + ((t & 7) >> 1), 1)

    xc2 = pick(lambda t, j: xc2b[j, pl.ds(t, 1), :])

    def pick_st(k):
        return jnp.where(first, jnp.broadcast_to(st[k][t1 >> 3, pl.ds(t1 & 7, 1), :], (8, 128)),
                         jnp.broadcast_to(st[k][t2 >> 3, pl.ds(t2 & 7, 1), :], (8, 128)))

    rs2 = pick_st(3)
    mm = pick_st(0) + pick_st(2)
    cb1r, sbr, gbr = mrow(5), mrow(6), mrow(7)
    h2 = [(xc2[j] * rs2) * cb1r[j] + sbr[j] for j in range(NJ)]
    x1s = [xc2[j] + mm for j in range(NJ)]
    hb = jnp.concatenate(h2, axis=1).astype(BF16)
    nt = (((1,), (1,)), ((), ()))
    cp_wg.wait()
    gg = lax.dot_general(hb, wgbuf[...], nt, preferred_element_type=F32)
    cp_wu.wait()
    uu = lax.dot_general(hb, wubuf[...], nt, preferred_element_type=F32)
    act = (gg * jax.nn.sigmoid(gg) * uu).astype(BF16)
    cp_wd.wait()
    for c in range(OCH):
        @pl.when(jnp.logical_and(c1 != c, c2 != c))
        def _():
            cp_out(c).start()
    yy = jnp.dot(act, wdbuf[...], preferred_element_type=F32)
    rsel = jnp.where(first[:, 0:1], m1, m2)
    yy = yy * jax.nn.sigmoid(rsel)
    for j in range(NJ):
        new = x1s[j] + gbr[j] * (h2[j] + yy[:, j * 128:(j + 1) * 128])
        bits = lax.bitcast_convert_type(_rb(new), U32)
        for (t, r) in ((t1, 0), (t2, 1)):
            old = o32[wrow(t, j), :]
            nb = bits[r:r + 1, :]
            o32[wrow(t, j), :] = jnp.where(
                (t & 1) == 1,
                (old & jnp.uint32(0x0000FFFF)) | nb,
                (old & jnp.uint32(0xFFFF0000)) | (nb >> 16))
    cp_out(c1).start()

    @pl.when(c2 != c1)
    def _():
        cp_out(c2).start()

    for c in range(OCH):
        cp_out(c).wait()


def _flat(x):
    return x.reshape(S // 8, 8, NJ, 128).transpose(0, 2, 1, 3).reshape(FL, 128)


def _unflat(y):
    return y.reshape(S // 8, NJ, 8, 128).transpose(0, 2, 1, 3).reshape(1, S, D)


@jax.jit
def pallas_adaLN_cond__ssm_conv_h3__moe_arch_mod__prompt_kernel(
    A_q: jax.Array,
    A_k: jax.Array,
    A_v: jax.Array,
    A_shift_k: jax.Array,
    A_ssm_k: jax.Array,
    A_ssm_D: jax.Array,
    B_x: jax.Array,
    B_w_r: jax.Array,
    B_w_gate: jax.Array,
    B_w_up: jax.Array,
    B_w_down: jax.Array,
    c: jax.Array,
    w_mod: jax.Array,
):
    del B_x
    args = (_flat(A_q), _flat(A_k), _flat(A_v), A_shift_k.T, A_ssm_k, A_ssm_D, B_w_r,
            B_w_gate.T, B_w_up.T, B_w_down, c, w_mod)
    V = pltpu.VMEM
    scratch = [
        V((FL + 48, 128), BF16),
        V((FL, 128), BF16),
        V((FL, 128), BF16),
        V((NJ, 128, S), BF16),
        V((D, 6 * D), BF16),
        V((F, D), BF16),
        V((F, D), BF16),
        V((F, D), BF16),
        V((4, D), BF16),
        V((D,), BF16),
        V((D,), BF16),
        V((1, D), BF16),
        V((NJ, 5, 8, 128), F32),
        V((NP, 256, 128), BF16),
        V((NP, 256, 128), BF16),
        V((NP, 2, 128, 128), BF16),
        V((S, 128), F32),
        V((NJ, 16, 256, 128), F32),
        V((NJ, 16, 256, 128), F32),
        V((2, 4, 256, 128), F32),
        V((16, 256, 128), F32),
        V((16, 256, 128), F32),
        V((NJ, S, 128), F32),
        V((NJ, S, 128), F32),
        V((NJ, S, 128), F32),
        V((NJ, S, 128), F32),
        V((S // 8, 8, 128), F32),
        V((S // 8, 8, 128), F32),
        V((S // 8, 8, 128), F32),
        V((S // 8, 8, 128), F32),
        V((FL, 128), BF16),
        V((8, 8, D), F32),
        pltpu.SemaphoreType.DMA((NSEM,)),
    ]
    out = pl.pallas_call(
        _kernel,
        out_shape=jax.ShapeDtypeStruct((FL, 128), BF16),
        in_specs=[pl.BlockSpec(memory_space=pl.ANY)] * len(args),
        out_specs=pl.BlockSpec(memory_space=pl.ANY),
        scratch_shapes=scratch,
        compiler_params=pltpu.CompilerParams(vmem_limit_bytes=100 * 1024 * 1024),
    )(*args)
    return _unflat(out)
```

```python
import math

import jax
import jax.numpy as jnp
from jax import lax
import jax.experimental.pallas as pl
import jax.experimental.pallas.tpu as pltpu

S = 2048
D = 640
F = 1728
NJ = D // 128
NA = 4
CH = S // NA
NP = 4
EPS = 1e-5
OCH = 4
WDCUT = 1472
EB = 8
NB = S // 8 // EB
QFIRST = 5
QSPLIT = 128 // EB + 3

F32 = jnp.float32
BF16 = jnp.bfloat16
U32 = jnp.uint32
I32 = jnp.int32

SEM_SK, SEM_DD, SEM_WR, SEM_C = 0, 1, 2, 3
SEM_SSM = 4
SEM_K = SEM_SSM + NJ
SEM_V = SEM_K + NA
SEM_WM = SEM_V + NA
SEM_Q = SEM_WM + 1
SEM_WG = SEM_Q + 3
SEM_WU = SEM_WG + 1
SEM_WD = SEM_WU + 1
SEM_OUT = SEM_WD + 2
NSEM = SEM_OUT + OCH


def _pack(x):
    return pltpu.bitcast(x.astype(BF16), U32)


def _unpack(w):
    return pltpu.bitcast(w, BF16)


def _cadd(x, y):
    return (x[0] + y[0], x[1] + y[1])


def _csub(x, y):
    return (x[0] - y[0], x[1] - y[1])


def _cadd_i(x, y):
    return (x[0] - y[1], x[1] + y[0])


def _csub_i(x, y):
    return (x[0] + y[1], x[1] - y[0])


def _cmul(x, y):
    return (x[0] * y[0] - x[1] * y[1], x[0] * y[1] + x[1] * y[0])


def _rb(x):
    return x.astype(BF16).astype(F32)


def _sum5(xs):
    return ((xs[0] + xs[1]) + (xs[2] + xs[3])) + xs[4]


def _cos_table(n):
    z = (jnp.abs(n - 1024) - 512).astype(F32) * (math.pi / 1024.0)
    z2 = z * z
    acc = jnp.full(z.shape, -1.0 / 39916800.0, F32)
    for cf in (1.0 / 362880.0, -1.0 / 5040.0, 1.0 / 120.0, -1.0 / 6.0, 1.0):
        acc = acc * z2 + cf
    return acc * z


def _mo(x, m):
    return x if isinstance(x, int) else pl.multiple_of(x, m)


def _lanes(j):
    return pl.ds(j * 128, 128)


def _kernel(q_hbm, k_hbm, v_hbm, sk_hbm, ssm_hbm, dd_hbm, wr_hbm, wg_hbm, wu_hbm,
            wd_hbm, c_hbm, wm_hbm, out_hbm,
            kbuf, vbuf, qbuf, sbuf, wmbuf, wgbuf, wubuf, wdbuf,
            skbuf, ddbuf, wrbuf, cbuf,
            prm, gf, gi, ktb, kf, vf, s1u, s1k, kraw, za, zb, ybuf,
            ring, st_m1, st_r1, st_m2, st_r2, obuf, mp, sems):
    def cp(src, dst, s):
        return pltpu.make_async_copy(src, dst, sems.at[s])

    def cp_ssm(j):
        return cp(ssm_hbm.at[pl.ds(_mo(j * 128, 128), 128), :], sbuf.at[j], SEM_SSM + j)

    def cp_k(a):
        return cp(k_hbm.at[0, pl.ds(_mo(a * CH, CH), CH), :],
                  kbuf.at[pl.ds(_mo(16 + a * CH, 16), CH), :], SEM_K + a)

    def cp_v(a):
        rows = pl.ds(_mo(a * CH, CH), CH)
        return cp(v_hbm.at[0, rows, :], vbuf.at[rows, :], SEM_V + a)

    def cp_q(h):
        cuts = (0, QFIRST * EB * 8, QSPLIT * EB * 8, S)
        rows = pl.ds(cuts[h], cuts[h + 1] - cuts[h])
        return cp(q_hbm.at[0, rows, :], qbuf.at[rows, :], SEM_Q + h)

    def cp_out(c):
        rows = pl.ds(_mo(c * (S // OCH), S // OCH), S // OCH)
        return cp(obuf.at[rows, :], out_hbm.at[0, rows, :], SEM_OUT + c)

    cp_sk = cp(sk_hbm, skbuf, SEM_SK)
    cp_dd = cp(dd_hbm, ddbuf, SEM_DD)
    cp_wr = cp(wr_hbm, wrbuf, SEM_WR)
    cp_c = cp(c_hbm, cbuf, SEM_C)
    cp_wm = cp(wm_hbm, wmbuf, SEM_WM)
    cp_wg = cp(wg_hbm, wgbuf, SEM_WG)
    cp_wu = cp(wu_hbm, wubuf, SEM_WU)
    cp_wda = cp(wd_hbm.at[pl.ds(0, WDCUT), :], wdbuf.at[pl.ds(0, WDCUT), :], SEM_WD)
    cp_wdb = cp(wd_hbm.at[pl.ds(WDCUT, F - WDCUT), :],
                wdbuf.at[pl.ds(WDCUT, F - WDCUT), :], SEM_WD + 1)

    cp_ssm(0).start()
    cp_dd.start()
    cp_sk.start()
    for j in range(1, NJ):
        cp_ssm(j).start()
    cp_wr.start()
    cp_c.start()
    kbuf[pl.ds(0, 16), :] = jnp.zeros((16, D), BF16)
    for a in range(NA):
        cp_k(a).start()
        cp_v(a).start()
    cp_wm.start()
    for h in range(3):
        cp_q(h).start()
    cp_wg.start()
    cp_wu.start()
    cp_wda.start()
    cp_wdb.start()

    for hb in range(2):
        rho = lax.broadcasted_iota(I32, (128, 128), 0) + 128 * hb
        col = lax.broadcasted_iota(I32, (128, 128), 1)
        n8 = ((rho >> 4) << 3) + (rho & 7)
        odd = 4 * n8 + (1 if hb == 0 else -253)
        n0 = odd * (4 * col) + ((rho >> 3) & 1) * 512
        for p in range(NP):
            tab = _cos_table((n0 + p * odd) & 2047)
            gf[p, pl.ds(64 * hb, 64), :] = _pack(tab)
            gi[p, hb] = _pack(tab.T * (2.0 / 1024.0))

    cp_sk.wait()
    cp_dd.wait()
    skf = skbuf[...].astype(F32)
    ddf = ddbuf[...].astype(F32).reshape(1, D)
    for j in range(NJ):
        for m in range(4):
            prm[j, m] = jnp.broadcast_to(skf[m:m + 1, j * 128:(j + 1) * 128], (8, 128))
        prm[j, 4] = jnp.broadcast_to(ddf[:, j * 128:(j + 1) * 128], (8, 128))

    def fft4(ys, g):
        x = [(y[16 * g:16 * g + 8, :], y[16 * g + 8:16 * g + 16, :]) for y in ys]
        e0, e1 = _cadd(x[0], x[2]), _cadd(x[1], x[3])
        d0, d1 = _csub(x[0], x[2]), _csub(x[1], x[3])
        return (_cadd(e0, e1), _csub_i(d0, d1), _csub(e0, e1), _cadd_i(d0, d1))

    def cst(ref, idx, g, val):
        ref[idx + (pl.ds(16 * g, 8), slice(None))] = val[0]
        ref[idx + (pl.ds(16 * g + 8, 8), slice(None))] = val[1]

    def cld(ref, idx, g):
        return (ref[idx + (pl.ds(16 * g, 8), slice(None))],
                ref[idx + (pl.ds(16 * g + 8, 8), slice(None))])

    def fwd_k(j, carry):
        cp_ssm(j).wait()
        for a in range(NA):
            ktb[pl.ds(CH * a, CH), :] = sbuf[j, :, pl.ds(CH * a, CH)].astype(F32).T
            ys = []
            for p in range(NP):
                kp = ktb[pl.ds(CH * a + p, 128, stride=4), :].astype(BF16)
                ys.append(jnp.dot(_unpack(gf[p]), kp, preferred_element_type=F32))
            for g in range(16):
                outs = fft4(ys, g)
                for f in range(4):
                    val = outs[f]
                    if a == 0:
                        val = (val[0] + prm[j, 4], val[1])
                    if 0 < a < NA - 1:
                        cst(kraw, (a - 1, f), g, val)
                    if a > 0:
                        prev = cld(s1k, (j, f), g) if a == 1 else cld(kraw, (a - 2, f), g)
                        val = _cadd_i(val, prev) if g < 8 else _csub_i(val, prev)
                    cst(s1k, (j, 4 * a + f), g, val)
        return carry

    lax.fori_loop(0, NJ, fwd_k, 0)

    def fwd_u(a, carry):
        cp_k(a).wait()
        cp_v(a).wait()
        kc = kbuf.at[pl.ds(_mo(a * CH, CH), CH + 16)]
        vc = vbuf.at[pl.ds(_mo(a * CH, CH), CH)]
        for j in range(NJ):
            for r in range(CH // 8 + 1):
                kf[j, pl.ds(8 * r, 8), :] = kc[pl.ds(8 + 8 * r, 8), _lanes(j)].astype(F32)
            for r in range(CH // 8):
                vf[j, pl.ds(8 * r, 8), :] = vc[pl.ds(8 * r, 8), _lanes(j)].astype(F32)
            ub = [[] for _ in range(NP)]
            for b in range(16):
                seq = [kf[j, pl.ds(32 * b + 5 + m, 8, stride=4), :] for m in range(7)]
                for p in range(NP):
                    ks = ((seq[p] * prm[j, 3] + seq[p + 1] * prm[j, 2])
                          + (seq[p + 2] * prm[j, 1] + seq[p + 3] * prm[j, 0]))
                    ub[p].append(ks * vf[j, pl.ds(32 * b + p, 8, stride=4), :])
            ys = [jnp.dot(_unpack(gf[p]), jnp.concatenate(ub[p], axis=0).astype(BF16),
                          preferred_element_type=F32) for p in range(NP)]
            for g in range(16):
                outs = fft4(ys, g)
                for f in range(4):
                    cst(s1u, (j, 4 * a + f), g, outs[f])
        return carry

    lax.fori_loop(0, NA, fwd_u, 0)

    def vpu_group(j, z_ref, g):
        for a in range(NA):
            zf = []
            for f in range(4):
                acc = None
                for jj in range(a + 1):
                    t = _cmul(cld(s1u, (j, 4 * (a - jj) + f), g), cld(s1k, (j, 4 * jj + f), g))
                    acc = t if acc is None else _cadd(acc, t)
                zf.append(acc)
            e0, e1 = _cadd(zf[0], zf[2]), _csub(zf[0], zf[2])
            o0, o1 = _cadd(zf[1], zf[3]), _csub(zf[1], zf[3])
            z = (_cadd(e0, o0), _cadd_i(e1, o1), _csub(e0, o0), _csub_i(e1, o1))
            for p in range(NP):
                cst(z_ref, (4 * a + p,), g, z[p])

    def inv_unit(j, z_ref, n):
        a, p = n // NP, n % NP
        lhs = jnp.concatenate([_unpack(gi[p, 0]), _unpack(gi[p, 1])], axis=1)
        ybuf[j, pl.ds(CH * a + p, 128, stride=4), :] = jnp.dot(
            lhs, z_ref[n].astype(BF16), preferred_element_type=F32)

    for g in range(16):
        vpu_group(0, za, g)

    def v_step(i, carry):
        j = 2 * i + 1
        for g in range(16):
            inv_unit(j - 1, za, g)
            vpu_group(j, zb, g)
        for g in range(16):
            inv_unit(j, zb, g)
            vpu_group(j + 1, za, g)
        return carry

    lax.fori_loop(0, (NJ - 1) // 2, v_step, 0)

    cp_c.wait()
    cp_wr.wait()
    cp_wm.wait()
    cp_q(0).wait()
    for n in range(16):
        inv_unit(NJ - 1, za, n)
    cf = cbuf[...].astype(F32)
    sc = (cf * jax.nn.sigmoid(cf)).astype(BF16)
    mod = jnp.dot(jnp.broadcast_to(sc, (16, D)), wmbuf[...],
                  preferred_element_type=F32)[0:8, :]
    mod = _rb(mod)
    sa, ca, ga, sb, cb, gb = [mod[:, i * D:(i + 1) * D] for i in range(6)]
    ca1 = _rb(1.0 + ca)
    cb1 = _rb(1.0 + cb)
    wrf = jnp.broadcast_to(wrbuf[...].astype(F32).reshape(1, D), (8, D))
    r0 = jnp.sum(wrf * sb, axis=-1, keepdims=True)
    sqd = math.sqrt(D)
    for i, val in enumerate((ga * ca1 * sqd, ga * sa, gb * cb1 * sqd, gb * sb,
                             wrf * cb1 * sqd, cb1 * sqd, sb, gb)):
        mp[i] = val

    def mrow(i):
        return [mp[i, :, _lanes(j)] for j in range(NJ)]

    lane = lax.broadcasted_iota(I32, (8, 128), 1)

    def rsum(xs):
        return jnp.broadcast_to(jnp.sum(_sum5(xs), axis=-1, keepdims=True), (8, 128))

    def brows(blk):
        return pl.ds(_mo(blk * EB * 8, EB * 8), EB * 8)

    def qtile(blk, i):
        qb = qbuf.at[brows(blk)]
        return [qb[pl.ds(8 * i, 8), _lanes(j)].astype(F32) for j in range(NJ)]

    def mix(xc, rs, y, a1, a0):
        return xc + ((xc * rs) * a1 + a0) * y

    def st1(blk, par, racc):
        for i in range(EB):
            st_m1[blk * EB + i] = rsum(qtile(blk, i)) * (1.0 / D)
        return racc

    def st2(blk, par, racc):
        for i in range(EB):
            m1 = st_m1[blk * EB + i]
            xc = [x - m1 for x in qtile(blk, i)]
            for j in range(NJ):
                ring[0, par, i, j] = xc[j]
            st_r1[blk * EB + i] = lax.rsqrt(rsum([c * c for c in xc]) + D * EPS)
        return racc

    def st3(blk, par, racc):
        a1, a0 = mrow(0), mrow(1)
        for i in range(EB):
            rs = st_r1[blk * EB + i]
            x1 = []
            for j in range(NJ):
                y = ybuf.at[j, brows(blk)][pl.ds(8 * i, 8), :]
                x1.append(mix(ring[0, par, i, j], rs, y, a1[j], a0[j]))
                ring[1, par, i, j] = x1[j]
            st_m2[blk * EB + i] = rsum(x1) * (1.0 / D)
        return racc

    def st4(blk, par, racc):
        w1 = mrow(4)
        for i in range(EB):
            m2 = st_m2[blk * EB + i]
            xc = [ring[1, par, i, j] - m2 for j in range(NJ)]
            for j in range(NJ):
                ring[2, par, i, j] = xc[j]
            rs = lax.rsqrt(rsum([c * c for c in xc]) + D * EPS)
            st_r2[blk * EB + i] = rs
            r = rsum([xc[j] * w1[j] for j in range(NJ)]) * rs
            racc = jnp.where(lane == ((blk * EB + i) & 127), r, racc)
        return racc

    def st5(blk, par, racc):
        b1, b0 = mrow(2), mrow(3)
        for i in range(EB):
            rs = st_r2[blk * EB + i]
            mm = st_m1[blk * EB + i] + st_m2[blk * EB + i]
            for j in range(NJ):
                obuf.at[brows(blk)][pl.ds(8 * i, 8), _lanes(j)] = (
                    ring[2, par, i, j] * (rs * b1[j] + 1.0) + (b0[j] + mm)).astype(BF16)
        return racc

    stages = (st1, st2, st3, st4, st5)

    def epi(n, par, racc):
        for k in reversed(range(len(stages))):
            if isinstance(n, int) and not 0 <= n - k < NB:
                continue
            racc = stages[k](n - k, (par + k) & 1, racc)
        return racc

    def epi2(i, racc):
        return epi(2 * i + 2, 0, epi(2 * i + 1, 1, racc))

    ra = jnp.zeros((8, 128), F32)
    for n in range(QFIRST):
        ra = epi(n, n & 1, ra)
    cp_q(1).wait()
    ra = lax.fori_loop(QFIRST // 2, QSPLIT // 2, epi2, ra)
    cp_q(2).wait()
    rb = lax.fori_loop(QSPLIT // 2, NB // 2 - 1, epi2, jnp.zeros((8, 128), F32))
    for n in range(NB - 1, NB + 4):
        rb = epi(n, n & 1, rb)

    bits = lax.bitcast_convert_type(_rb(jnp.concatenate([ra, rb], axis=1) + r0), I32)
    tok = (lax.broadcasted_iota(I32, (8, 256), 1) * 8
           + lax.broadcasted_iota(I32, (8, 256), 0))
    flip = lambda x: x ^ ((x >> 31) & 0x7FFF0000)
    key = flip(bits) | (S - 1 - tok)

    def amax(x):
        x = jnp.maximum(x[:, :128], x[:, 128:])
        return jnp.max(jnp.max(x, axis=0, keepdims=True), axis=1, keepdims=True)

    k1 = amax(key)
    k2 = amax(jnp.where(key == k1, jnp.iinfo(jnp.int32).min, key))
    t1 = jnp.clip(S - 1 - (k1[0, 0] & 0xFFFF), 0, S - 1)
    t2 = jnp.clip(S - 1 - (k2[0, 0] & 0xFFFF), 0, S - 1)
    m1, m2 = [lax.bitcast_convert_type(flip(kk & -65536), F32) for kk in (k1, k2)]
    c1 = t1 // (S // OCH)
    c2 = t2 // (S // OCH)

    first = lax.broadcasted_iota(I32, (8, 128), 0) == 0

    def pick(get):
        return jnp.where(first, jnp.broadcast_to(get(t1), (8, 128)),
                         jnp.broadcast_to(get(t2), (8, 128)))

    def pick_st(ref):
        return pick(lambda t: ref[t >> 3, pl.ds(t & 7, 1), :])

    rowi = lax.broadcasted_iota(I32, (16, D), 0)

    def blk16(t):
        return pl.ds(pl.multiple_of((t >> 4) << 4, 16), 16)

    def qrow(t):
        return jnp.sum(jnp.where(rowi == (t & 15), qbuf[blk16(t), :].astype(F32), 0.0),
                       axis=0, keepdims=True)

    q1, q2 = qrow(t1), qrow(t2)
    m1s, m2s, rs1, rs2 = pick_st(st_m1), pick_st(st_m2), pick_st(st_r1), pick_st(st_r2)
    a1, a0 = mrow(0), mrow(1)
    xc2 = []
    for j in range(NJ):
        xq = jnp.where(first, jnp.broadcast_to(q1[:, j * 128:(j + 1) * 128], (8, 128)),
                       jnp.broadcast_to(q2[:, j * 128:(j + 1) * 128], (8, 128)))
        y = pick(lambda t: ybuf[j, pl.ds(t, 1), :])
        xc2.append(mix(xq - m1s, rs1, y, a1[j], a0[j]) - m2s)
    mm = m1s + m2s
    cb1r, sbr, gbr = mrow(5), mrow(6), mrow(7)
    h2 = [(xc2[j] * rs2) * cb1r[j] + sbr[j] for j in range(NJ)]
    hb = jnp.concatenate(h2, axis=1).astype(BF16)
    nt = (((1,), (1,)), ((), ()))
    cp_wg.wait()
    gg = lax.dot_general(hb, wgbuf[...], nt, preferred_element_type=F32)
    cp_wda.wait()
    for c in range(OCH):
        @pl.when(jnp.logical_and(c1 != c, c2 != c))
        def _():
            cp_out(c).start()
    cp_wu.wait()
    uu = lax.dot_general(hb, wubuf[...], nt, preferred_element_type=F32)
    act = (gg * jax.nn.sigmoid(gg) * uu).astype(BF16)
    cp_wdb.wait()
    yy = jnp.dot(act, wdbuf[...], preferred_element_type=F32)
    yy = yy * jax.nn.sigmoid(jnp.where(first[:, 0:1], m1, m2))
    new = jnp.concatenate(
        [(xc2[j] + mm) + gbr[j] * (h2[j] + yy[:, j * 128:(j + 1) * 128]) for j in range(NJ)],
        axis=1)
    for (t, r) in ((t1, 0), (t2, 1)):
        blk = blk16(t)
        obuf[blk, :] = jnp.where(rowi == (t & 15),
                                 jnp.broadcast_to(new[r:r + 1, :], (16, D)),
                                 obuf[blk, :].astype(F32)).astype(BF16)
    cp_out(c1).start()

    @pl.when(c2 != c1)
    def _():
        cp_out(c2).start()

    for c in range(OCH):
        cp_out(c).wait()


@jax.jit
def pallas_adaLN_cond__ssm_conv_h3__moe_arch_mod__prompt_kernel(
    A_q: jax.Array,
    A_k: jax.Array,
    A_v: jax.Array,
    A_shift_k: jax.Array,
    A_ssm_k: jax.Array,
    A_ssm_D: jax.Array,
    B_x: jax.Array,
    B_w_r: jax.Array,
    B_w_gate: jax.Array,
    B_w_up: jax.Array,
    B_w_down: jax.Array,
    c: jax.Array,
    w_mod: jax.Array,
):
    del B_x
    args = (A_q, A_k, A_v, A_shift_k.T, A_ssm_k, A_ssm_D, B_w_r,
            B_w_gate.T, B_w_up.T, B_w_down, c, w_mod)
    V = pltpu.VMEM
    scratch = [
        V((S + 16, D), BF16),
        V((S, D), BF16),
        V((S, D), BF16),
        V((NJ, 128, S), BF16),
        V((D, 6 * D), BF16),
        V((F, D), BF16),
        V((F, D), BF16),
        V((F, D), BF16),
        V((4, D), BF16),
        V((D,), BF16),
        V((D,), BF16),
        V((1, D), BF16),
        V((NJ, 5, 8, 128), F32),
        V((NP, 128, 128), U32),
        V((NP, 2, 64, 128), U32),
        V((S, 128), F32),
        V((NJ, CH + 8, 128), F32),
        V((NJ, CH, 128), F32),
        V((NJ, 16, 256, 128), F32),
        V((NJ, 16, 256, 128), F32),
        V((2, 4, 256, 128), F32),
        V((16, 256, 128), F32),
        V((16, 256, 128), F32),
        V((NJ, S, 128), F32),
        V((3, 2, EB, NJ, 8, 128), F32),
        V((S // 8, 8, 128), F32),
        V((S // 8, 8, 128), F32),
        V((S // 8, 8, 128), F32),
        V((S // 8, 8, 128), F32),
        V((S, D), BF16),
        V((8, 8, D), F32),
        pltpu.SemaphoreType.DMA((NSEM,)),
    ]
    return pl.pallas_call(
        _kernel,
        out_shape=jax.ShapeDtypeStruct((1, S, D), BF16),
        in_specs=[pl.BlockSpec(memory_space=pl.ANY)] * len(args),
        out_specs=pl.BlockSpec(memory_space=pl.ANY),
        scratch_shapes=scratch,
        compiler_params=pltpu.CompilerParams(vmem_limit_bytes=100 * 1024 * 1024),
    )(*args)
```

```python
import math

import jax
import jax.numpy as jnp
from jax import lax
import jax.experimental.pallas as pl
import jax.experimental.pallas.tpu as pltpu

S = 2048
D = 640
F = 1728
NJ = D // 128
NA = 4
CH = S // NA
NP = 4
EPS = 1e-5
OCH = 8
WDCUT = 1472
EB = 8
NB = S // 8 // EB
QFIRST = 5
QSPLIT = 128 // EB + 3

F32 = jnp.float32
BF16 = jnp.bfloat16
U32 = jnp.uint32
I32 = jnp.int32

SEM_SK, SEM_DD, SEM_WR, SEM_C = 0, 1, 2, 3
SEM_SSM = 4
SEM_K = SEM_SSM + NJ
SEM_V = SEM_K + NA
SEM_WM = SEM_V + NA
SEM_Q = SEM_WM + 1
SEM_WG = SEM_Q + 3
SEM_WU = SEM_WG + 1
SEM_WD = SEM_WU + 1
SEM_OUT = SEM_WD + 2
NSEM = SEM_OUT + OCH


def _pack(x):
    return pltpu.bitcast(x.astype(BF16), U32)


def _unpack(w):
    return pltpu.bitcast(w, BF16)


def _cadd(x, y):
    return (x[0] + y[0], x[1] + y[1])


def _csub(x, y):
    return (x[0] - y[0], x[1] - y[1])


def _cadd_i(x, y):
    return (x[0] - y[1], x[1] + y[0])


def _csub_i(x, y):
    return (x[0] + y[1], x[1] - y[0])


def _cmul(x, y):
    return (x[0] * y[0] - x[1] * y[1], x[0] * y[1] + x[1] * y[0])


def _rb(x):
    return x.astype(BF16).astype(F32)


def _sum5(xs):
    return ((xs[0] + xs[1]) + (xs[2] + xs[3])) + xs[4]


def _cos_table(n):
    z = (jnp.abs(n - 1024) - 512).astype(F32) * (math.pi / 1024.0)
    z2 = z * z
    acc = jnp.full(z.shape, -1.0 / 39916800.0, F32)
    for cf in (1.0 / 362880.0, -1.0 / 5040.0, 1.0 / 120.0, -1.0 / 6.0, 1.0):
        acc = acc * z2 + cf
    return acc * z


def _mo(x, m):
    return x if isinstance(x, int) else pl.multiple_of(x, m)


def _lanes(j):
    return pl.ds(j * 128, 128)


def _kernel(q_hbm, k_hbm, v_hbm, sk_hbm, ssm_hbm, dd_hbm, wr_hbm, wg_hbm, wu_hbm,
            wd_hbm, c_hbm, wm_hbm, out_hbm,
            kbuf, vbuf, qbuf, sbuf, wmbuf, wgbuf, wubuf, wdbuf,
            skbuf, ddbuf, wrbuf, cbuf,
            prm, gf, gi, ktb, kf, vf, s1u, s1k, kraw, za, zb, ybuf,
            ring, st_m1, st_r1, st_m2, st_r2, obuf, mp, sems):
    def cp(src, dst, s):
        return pltpu.make_async_copy(src, dst, sems.at[s])

    def cp_ssm(j):
        return cp(ssm_hbm.at[pl.ds(_mo(j * 128, 128), 128), :], sbuf.at[j], SEM_SSM + j)

    def cp_k(a):
        return cp(k_hbm.at[0, pl.ds(_mo(a * CH, CH), CH), :],
                  kbuf.at[pl.ds(_mo(16 + a * CH, 16), CH), :], SEM_K + a)

    def cp_v(a):
        rows = pl.ds(_mo(a * CH, CH), CH)
        return cp(v_hbm.at[0, rows, :], vbuf.at[rows, :], SEM_V + a)

    def cp_q(h):
        cuts = (0, QFIRST * EB * 8, QSPLIT * EB * 8, S)
        rows = pl.ds(cuts[h], cuts[h + 1] - cuts[h])
        return cp(q_hbm.at[0, rows, :], qbuf.at[rows, :], SEM_Q + h)

    def cp_out(c):
        rows = pl.ds(_mo(c * (S // OCH), S // OCH), S // OCH)
        return cp(obuf.at[rows, :], out_hbm.at[0, rows, :], SEM_OUT + c)

    cp_sk = cp(sk_hbm, skbuf, SEM_SK)
    cp_dd = cp(dd_hbm, ddbuf, SEM_DD)
    cp_wr = cp(wr_hbm, wrbuf, SEM_WR)
    cp_c = cp(c_hbm, cbuf, SEM_C)
    cp_wm = cp(wm_hbm, wmbuf, SEM_WM)
    cp_wg = cp(wg_hbm, wgbuf, SEM_WG)
    cp_wu = cp(wu_hbm, wubuf, SEM_WU)
    cp_wda = cp(wd_hbm.at[pl.ds(0, WDCUT), :], wdbuf.at[pl.ds(0, WDCUT), :], SEM_WD)
    cp_wdb = cp(wd_hbm.at[pl.ds(WDCUT, F - WDCUT), :],
                wdbuf.at[pl.ds(WDCUT, F - WDCUT), :], SEM_WD + 1)

    cp_ssm(0).start()
    cp_dd.start()
    cp_sk.start()
    for j in range(1, NJ):
        cp_ssm(j).start()
    cp_wr.start()
    cp_c.start()
    kbuf[pl.ds(0, 16), :] = jnp.zeros((16, D), BF16)
    for a in range(NA):
        cp_k(a).start()
        cp_v(a).start()
    cp_wm.start()
    for h in range(3):
        cp_q(h).start()
    cp_wg.start()
    cp_wu.start()
    cp_wda.start()
    cp_wdb.start()

    for hb in range(2):
        rho = lax.broadcasted_iota(I32, (128, 128), 0) + 128 * hb
        col = lax.broadcasted_iota(I32, (128, 128), 1)
        n8 = ((rho >> 4) << 3) + (rho & 7)
        odd = 4 * n8 + (1 if hb == 0 else -253)
        n0 = odd * (4 * col) + ((rho >> 3) & 1) * 512
        for p in range(NP):
            tab = _cos_table((n0 + p * odd) & 2047)
            gf[p, pl.ds(64 * hb, 64), :] = _pack(tab)
            gi[p, hb] = _pack(tab.T * (2.0 / 1024.0))

    cp_sk.wait()
    cp_dd.wait()
    skf = skbuf[...].astype(F32)
    ddf = ddbuf[...].astype(F32).reshape(1, D)
    for j in range(NJ):
        for m in range(4):
            prm[j, m] = jnp.broadcast_to(skf[m:m + 1, j * 128:(j + 1) * 128], (8, 128))
        prm[j, 4] = jnp.broadcast_to(ddf[:, j * 128:(j + 1) * 128], (8, 128))

    def fft4(ys, g):
        x = [(y[16 * g:16 * g + 8, :], y[16 * g + 8:16 * g + 16, :]) for y in ys]
        e0, e1 = _cadd(x[0], x[2]), _cadd(x[1], x[3])
        d0, d1 = _csub(x[0], x[2]), _csub(x[1], x[3])
        return (_cadd(e0, e1), _csub_i(d0, d1), _csub(e0, e1), _cadd_i(d0, d1))

    def cst(ref, idx, g, val):
        ref[idx + (pl.ds(16 * g, 8), slice(None))] = val[0]
        ref[idx + (pl.ds(16 * g + 8, 8), slice(None))] = val[1]

    def cld(ref, idx, g):
        return (ref[idx + (pl.ds(16 * g, 8), slice(None))],
                ref[idx + (pl.ds(16 * g + 8, 8), slice(None))])

    def fwd_k(j, carry):
        cp_ssm(j).wait()
        for a in range(NA):
            ktb[pl.ds(CH * a, CH), :] = sbuf[j, :, pl.ds(CH * a, CH)].astype(F32).T
            ys = []
            for p in range(NP):
                kp = ktb[pl.ds(CH * a + p, 128, stride=4), :].astype(BF16)
                ys.append(jnp.dot(_unpack(gf[p]), kp, preferred_element_type=F32))
            for g in range(16):
                outs = fft4(ys, g)
                for f in range(4):
                    val = outs[f]
                    if a == 0:
                        val = (val[0] + prm[j, 4], val[1])
                    if 0 < a < NA - 1:
                        cst(kraw, (a - 1, f), g, val)
                    if a > 0:
                        prev = cld(s1k, (j, f), g) if a == 1 else cld(kraw, (a - 2, f), g)
                        val = _cadd_i(val, prev) if g < 8 else _csub_i(val, prev)
                    cst(s1k, (j, 4 * a + f), g, val)
        return carry

    lax.fori_loop(0, NJ, fwd_k, 0)

    def fwd_u(a, carry):
        cp_k(a).wait()
        cp_v(a).wait()
        kc = kbuf.at[pl.ds(_mo(a * CH, CH), CH + 16)]
        vc = vbuf.at[pl.ds(_mo(a * CH, CH), CH)]
        for j in range(NJ):
            for r in range(CH // 8 + 1):
                kf[j, pl.ds(8 * r, 8), :] = kc[pl.ds(8 + 8 * r, 8), _lanes(j)].astype(F32)
            for r in range(CH // 8):
                vf[j, pl.ds(8 * r, 8), :] = vc[pl.ds(8 * r, 8), _lanes(j)].astype(F32)
            ub = [[] for _ in range(NP)]
            for b in range(16):
                seq = [kf[j, pl.ds(32 * b + 5 + m, 8, stride=4), :] for m in range(7)]
                for p in range(NP):
                    ks = ((seq[p] * prm[j, 3] + seq[p + 1] * prm[j, 2])
                          + (seq[p + 2] * prm[j, 1] + seq[p + 3] * prm[j, 0]))
                    ub[p].append(ks * vf[j, pl.ds(32 * b + p, 8, stride=4), :])
            ys = [jnp.dot(_unpack(gf[p]), jnp.concatenate(ub[p], axis=0).astype(BF16),
                          preferred_element_type=F32) for p in range(NP)]
            for g in range(16):
                outs = fft4(ys, g)
                for f in range(4):
                    cst(s1u, (j, 4 * a + f), g, outs[f])
        return carry

    lax.fori_loop(0, NA, fwd_u, 0)

    def vpu_group(j, z_ref, g):
        for a in range(NA):
            zf = []
            for f in range(4):
                acc = None
                for jj in range(a + 1):
                    t = _cmul(cld(s1u, (j, 4 * (a - jj) + f), g), cld(s1k, (j, 4 * jj + f), g))
                    acc = t if acc is None else _cadd(acc, t)
                zf.append(acc)
            e0, e1 = _cadd(zf[0], zf[2]), _csub(zf[0], zf[2])
            o0, o1 = _cadd(zf[1], zf[3]), _csub(zf[1], zf[3])
            z = (_cadd(e0, o0), _cadd_i(e1, o1), _csub(e0, o0), _csub_i(e1, o1))
            for p in range(NP):
                cst(z_ref, (4 * a + p,), g, z[p])

    def inv_unit(j, z_ref, n):
        a, p = n // NP, n % NP
        lhs = jnp.concatenate([_unpack(gi[p, 0]), _unpack(gi[p, 1])], axis=1)
        ybuf[j, pl.ds(CH * a + p, 128, stride=4), :] = jnp.dot(
            lhs, z_ref[n].astype(BF16), preferred_element_type=F32)

    for g in range(16):
        vpu_group(0, za, g)

    def v_step(i, carry):
        j = 2 * i + 1
        for g in range(16):
            inv_unit(j - 1, za, g)
            vpu_group(j, zb, g)
        for g in range(16):
            inv_unit(j, zb, g)
            vpu_group(j + 1, za, g)
        return carry

    lax.fori_loop(0, (NJ - 1) // 2, v_step, 0)

    cp_c.wait()
    cp_wr.wait()
    cp_wm.wait()
    cp_q(0).wait()
    for n in range(16):
        inv_unit(NJ - 1, za, n)
    cf = cbuf[...].astype(F32)
    sc = (cf * jax.nn.sigmoid(cf)).astype(BF16)
    mod = jnp.dot(jnp.broadcast_to(sc, (16, D)), wmbuf[...],
                  preferred_element_type=F32)[0:8, :]
    mod = _rb(mod)
    sa, ca, ga, sb, cb, gb = [mod[:, i * D:(i + 1) * D] for i in range(6)]
    ca1 = _rb(1.0 + ca)
    cb1 = _rb(1.0 + cb)
    wrf = jnp.broadcast_to(wrbuf[...].astype(F32).reshape(1, D), (8, D))
    r0 = jnp.sum(wrf * sb, axis=-1, keepdims=True)
    sqd = math.sqrt(D)
    for i, val in enumerate((ga * ca1 * sqd, ga * sa, gb * cb1 * sqd, gb * sb,
                             wrf * cb1 * sqd, cb1 * sqd, sb, gb)):
        mp[i] = val

    def mrow(i):
        return [mp[i, :, _lanes(j)] for j in range(NJ)]

    lane = lax.broadcasted_iota(I32, (8, 128), 1)

    def rsum(xs):
        return jnp.broadcast_to(jnp.sum(_sum5(xs), axis=-1, keepdims=True), (8, 128))

    def brows(blk):
        return pl.ds(_mo(blk * EB * 8, EB * 8), EB * 8)

    def qtile(blk, i):
        qb = qbuf.at[brows(blk)]
        return [qb[pl.ds(8 * i, 8), _lanes(j)].astype(F32) for j in range(NJ)]

    def mix(xc, rs, y, a1, a0):
        return xc + ((xc * rs) * a1 + a0) * y

    def st1(blk, par, racc):
        for i in range(EB):
            st_m1[blk * EB + i] = rsum(qtile(blk, i)) * (1.0 / D)
        return racc

    def st2(blk, par, racc):
        for i in range(EB):
            m1 = st_m1[blk * EB + i]
            xc = [x - m1 for x in qtile(blk, i)]
            for j in range(NJ):
                ring[0, par, i, j] = xc[j]
            st_r1[blk * EB + i] = lax.rsqrt(rsum([c * c for c in xc]) + D * EPS)
        return racc

    def st3(blk, par, racc):
        a1, a0 = mrow(0), mrow(1)
        for i in range(EB):
            rs = st_r1[blk * EB + i]
            x1 = []
            for j in range(NJ):
                y = ybuf.at[j, brows(blk)][pl.ds(8 * i, 8), :]
                x1.append(mix(ring[0, par, i, j], rs, y, a1[j], a0[j]))
                ring[1, par, i, j] = x1[j]
            st_m2[blk * EB + i] = rsum(x1) * (1.0 / D)
        return racc

    def st4(blk, par, racc):
        w1 = mrow(4)
        for i in range(EB):
            m2 = st_m2[blk * EB + i]
            xc = [ring[1, par, i, j] - m2 for j in range(NJ)]
            for j in range(NJ):
                ring[2, par, i, j] = xc[j]
            rs = lax.rsqrt(rsum([c * c for c in xc]) + D * EPS)
            st_r2[blk * EB + i] = rs
            r = rsum([xc[j] * w1[j] for j in range(NJ)]) * rs
            racc = jnp.where(lane == ((blk * EB + i) & 127), r, racc)
        return racc

    def st5(blk, par, racc):
        b1, b0 = mrow(2), mrow(3)
        for i in range(EB):
            rs = st_r2[blk * EB + i]
            mm = st_m1[blk * EB + i] + st_m2[blk * EB + i]
            for j in range(NJ):
                obuf.at[brows(blk)][pl.ds(8 * i, 8), _lanes(j)] = (
                    ring[2, par, i, j] * (rs * b1[j] + 1.0) + (b0[j] + mm)).astype(BF16)
        return racc

    stages = (st1, st2, st3, st4, st5)

    def epi(n, par, racc):
        for k in reversed(range(len(stages))):
            if isinstance(n, int) and not 0 <= n - k < NB:
                continue
            racc = stages[k](n - k, (par + k) & 1, racc)
        return racc

    def epi2(i, racc):
        return epi(2 * i + 2, 0, epi(2 * i + 1, 1, racc))

    ra = jnp.zeros((8, 128), F32)
    for n in range(QFIRST):
        ra = epi(n, n & 1, ra)
    cp_q(1).wait()
    ra = lax.fori_loop(QFIRST // 2, QSPLIT // 2, epi2, ra)
    cp_q(2).wait()
    rb = lax.fori_loop(QSPLIT // 2, NB // 2 - 1, epi2, jnp.zeros((8, 128), F32))
    for n in range(NB - 1, NB + 4):
        rb = epi(n, n & 1, rb)

    bits = lax.bitcast_convert_type(_rb(jnp.concatenate([ra, rb], axis=1) + r0), I32)
    tok = (lax.broadcasted_iota(I32, (8, 256), 1) * 8
           + lax.broadcasted_iota(I32, (8, 256), 0))
    flip = lambda x: x ^ ((x >> 31) & 0x7FFF0000)
    key = flip(bits) | (S - 1 - tok)

    def amax(x):
        x = jnp.maximum(x[:, :128], x[:, 128:])
        return jnp.max(jnp.max(x, axis=0, keepdims=True), axis=1, keepdims=True)

    k1 = amax(key)
    k2 = amax(jnp.where(key == k1, jnp.iinfo(jnp.int32).min, key))
    t1 = jnp.clip(S - 1 - (k1[0, 0] & 0xFFFF), 0, S - 1)
    t2 = jnp.clip(S - 1 - (k2[0, 0] & 0xFFFF), 0, S - 1)
    m1, m2 = [lax.bitcast_convert_type(flip(kk & -65536), F32) for kk in (k1, k2)]
    c1 = t1 // (S // OCH)
    c2 = t2 // (S // OCH)

    first = lax.broadcasted_iota(I32, (8, 128), 0) == 0

    def pick(get):
        return jnp.where(first, jnp.broadcast_to(get(t1), (8, 128)),
                         jnp.broadcast_to(get(t2), (8, 128)))

    def pick_st(ref):
        return pick(lambda t: ref[t >> 3, pl.ds(t & 7, 1), :])

    rowi = lax.broadcasted_iota(I32, (16, D), 0)

    def blk16(t):
        return pl.ds(pl.multiple_of((t >> 4) << 4, 16), 16)

    def qrow(t):
        return jnp.sum(jnp.where(rowi == (t & 15), qbuf[blk16(t), :].astype(F32), 0.0),
                       axis=0, keepdims=True)

    q1, q2 = qrow(t1), qrow(t2)
    m1s, m2s, rs1, rs2 = pick_st(st_m1), pick_st(st_m2), pick_st(st_r1), pick_st(st_r2)
    a1, a0 = mrow(0), mrow(1)
    xc2 = []
    for j in range(NJ):
        xq = jnp.where(first, jnp.broadcast_to(q1[:, j * 128:(j + 1) * 128], (8, 128)),
                       jnp.broadcast_to(q2[:, j * 128:(j + 1) * 128], (8, 128)))
        y = pick(lambda t: ybuf[j, pl.ds(t, 1), :])
        xc2.append(mix(xq - m1s, rs1, y, a1[j], a0[j]) - m2s)
    mm = m1s + m2s
    cb1r, sbr, gbr = mrow(5), mrow(6), mrow(7)
    h2 = [(xc2[j] * rs2) * cb1r[j] + sbr[j] for j in range(NJ)]
    hb = jnp.concatenate(h2, axis=1).astype(BF16)
    nt = (((1,), (1,)), ((), ()))
    cp_wg.wait()
    gg = lax.dot_general(hb, wgbuf[...], nt, preferred_element_type=F32)
    cp_wda.wait()
    for c in range(OCH):
        @pl.when(jnp.logical_and(c1 != c, c2 != c))
        def _():
            cp_out(c).start(priority=c % 2)
    cp_wu.wait()
    uu = lax.dot_general(hb, wubuf[...], nt, preferred_element_type=F32)
    act = (gg * jax.nn.sigmoid(gg) * uu).astype(BF16)
    cp_wdb.wait()
    yy = jnp.dot(act, wdbuf[...], preferred_element_type=F32)
    yy = yy * jax.nn.sigmoid(jnp.where(first[:, 0:1], m1, m2))
    new = jnp.concatenate(
        [(xc2[j] + mm) + gbr[j] * (h2[j] + yy[:, j * 128:(j + 1) * 128]) for j in range(NJ)],
        axis=1)
    for (t, r) in ((t1, 0), (t2, 1)):
        blk = blk16(t)
        obuf[blk, :] = jnp.where(rowi == (t & 15),
                                 jnp.broadcast_to(new[r:r + 1, :], (16, D)),
                                 obuf[blk, :].astype(F32)).astype(BF16)
    cp_out(c1).start()

    @pl.when(c2 != c1)
    def _():
        cp_out(c2).start()

    for c in range(OCH):
        cp_out(c).wait()


@jax.jit
def pallas_adaLN_cond__ssm_conv_h3__moe_arch_mod__prompt_kernel(
    A_q: jax.Array,
    A_k: jax.Array,
    A_v: jax.Array,
    A_shift_k: jax.Array,
    A_ssm_k: jax.Array,
    A_ssm_D: jax.Array,
    B_x: jax.Array,
    B_w_r: jax.Array,
    B_w_gate: jax.Array,
    B_w_up: jax.Array,
    B_w_down: jax.Array,
    c: jax.Array,
    w_mod: jax.Array,
):
    del B_x
    args = (A_q, A_k, A_v, A_shift_k.T, A_ssm_k, A_ssm_D, B_w_r,
            B_w_gate.T, B_w_up.T, B_w_down, c, w_mod)
    V = pltpu.VMEM
    scratch = [
        V((S + 16, D), BF16),
        V((S, D), BF16),
        V((S, D), BF16),
        V((NJ, 128, S), BF16),
        V((D, 6 * D), BF16),
        V((F, D), BF16),
        V((F, D), BF16),
        V((F, D), BF16),
        V((4, D), BF16),
        V((D,), BF16),
        V((D,), BF16),
        V((1, D), BF16),
        V((NJ, 5, 8, 128), F32),
        V((NP, 128, 128), U32),
        V((NP, 2, 64, 128), U32),
        V((S, 128), F32),
        V((NJ, CH + 8, 128), F32),
        V((NJ, CH, 128), F32),
        V((NJ, 16, 256, 128), F32),
        V((NJ, 16, 256, 128), F32),
        V((2, 4, 256, 128), F32),
        V((16, 256, 128), F32),
        V((16, 256, 128), F32),
        V((NJ, S, 128), F32),
        V((3, 2, EB, NJ, 8, 128), F32),
        V((S // 8, 8, 128), F32),
        V((S // 8, 8, 128), F32),
        V((S // 8, 8, 128), F32),
        V((S // 8, 8, 128), F32),
        V((S, D), BF16),
        V((8, 8, D), F32),
        pltpu.SemaphoreType.DMA((NSEM,)),
    ]
    return pl.pallas_call(
        _kernel,
        out_shape=jax.ShapeDtypeStruct((1, S, D), BF16),
        in_specs=[pl.BlockSpec(memory_space=pl.ANY)] * len(args),
        out_specs=pl.BlockSpec(memory_space=pl.ANY),
        scratch_shapes=scratch,
        compiler_params=pltpu.CompilerParams(vmem_limit_bytes=100 * 1024 * 1024,
                                             disable_semaphore_checks=True),
    )(*args)
```

```python
import math

import jax
import jax.numpy as jnp
from jax import lax
import jax.experimental.pallas as pl
import jax.experimental.pallas.tpu as pltpu

S = 2048
D = 640
F = 1728
NJ = D // 128
NA = 4
CH = S // NA
NP = 4
EPS = 1e-5
OCH = 8
WDCUT = 1472
EB = 8
NB = S // 8 // EB
QFIRST = 5
QSPLIT = 128 // EB + 3

F32 = jnp.float32
BF16 = jnp.bfloat16
U32 = jnp.uint32
I32 = jnp.int32

SEM_SK, SEM_DD, SEM_WR, SEM_C = 0, 1, 2, 3
SEM_SSM = 4
SEM_K = SEM_SSM + NJ
SEM_V = SEM_K + NA
SEM_WM = SEM_V + NA
SEM_Q = SEM_WM + 1
SEM_WG = SEM_Q + 3
SEM_WU = SEM_WG + 1
SEM_WD = SEM_WU + 1
SEM_OUT = SEM_WD + 2
NSEM = SEM_OUT + OCH


def _pack(x):
    return pltpu.bitcast(x.astype(BF16), U32)


def _unpack(w):
    return pltpu.bitcast(w, BF16)


def _cadd(x, y):
    return (x[0] + y[0], x[1] + y[1])


def _csub(x, y):
    return (x[0] - y[0], x[1] - y[1])


def _cadd_i(x, y):
    return (x[0] - y[1], x[1] + y[0])


def _csub_i(x, y):
    return (x[0] + y[1], x[1] - y[0])


def _cmul(x, y):
    return (x[0] * y[0] - x[1] * y[1], x[0] * y[1] + x[1] * y[0])


def _rb(x):
    return x.astype(BF16).astype(F32)


def _sigmoid(x):
    return _rb(1.0 / _rb(1.0 + _rb(jnp.exp(-x))))


def _sum5(xs):
    return ((xs[0] + xs[1]) + (xs[2] + xs[3])) + xs[4]


def _cos_table(n):
    z = (jnp.abs(n - 1024) - 512).astype(F32) * (math.pi / 1024.0)
    z2 = z * z
    acc = jnp.full(z.shape, -1.0 / 39916800.0, F32)
    for cf in (1.0 / 362880.0, -1.0 / 5040.0, 1.0 / 120.0, -1.0 / 6.0, 1.0):
        acc = acc * z2 + cf
    return acc * z


def _mo(x, m):
    return x if isinstance(x, int) else pl.multiple_of(x, m)


def _lanes(j):
    return pl.ds(j * 128, 128)


def _kernel(q_hbm, k_hbm, v_hbm, sk_hbm, ssm_hbm, dd_hbm, wr_hbm, wg_hbm, wu_hbm,
            wd_hbm, c_hbm, wm_hbm, out_hbm,
            kbuf, vbuf, qbuf, sbuf, wmbuf, wgbuf, wubuf, wdbuf,
            skbuf, ddbuf, wrbuf, cbuf,
            prm, gf, gi, ktb, kf, vf, s1u, s1k, kraw, za, zb, ybuf,
            ring, st_m1, st_r1, st_m2, st_r2, obuf, mp, sems):
    def cp(src, dst, s):
        return pltpu.make_async_copy(src, dst, sems.at[s])

    def cp_ssm(j):
        return cp(ssm_hbm.at[pl.ds(_mo(j * 128, 128), 128), :], sbuf.at[j], SEM_SSM + j)

    def cp_k(a):
        return cp(k_hbm.at[0, pl.ds(_mo(a * CH, CH), CH), :],
                  kbuf.at[pl.ds(_mo(16 + a * CH, 16), CH), :], SEM_K + a)

    def cp_v(a):
        rows = pl.ds(_mo(a * CH, CH), CH)
        return cp(v_hbm.at[0, rows, :], vbuf.at[rows, :], SEM_V + a)

    def cp_q(h):
        cuts = (0, QFIRST * EB * 8, QSPLIT * EB * 8, S)
        rows = pl.ds(cuts[h], cuts[h + 1] - cuts[h])
        return cp(q_hbm.at[0, rows, :], qbuf.at[rows, :], SEM_Q + h)

    def cp_out(c):
        rows = pl.ds(_mo(c * (S // OCH), S // OCH), S // OCH)
        return cp(obuf.at[rows, :], out_hbm.at[0, rows, :], SEM_OUT + c)

    cp_sk = cp(sk_hbm, skbuf, SEM_SK)
    cp_dd = cp(dd_hbm, ddbuf, SEM_DD)
    cp_wr = cp(wr_hbm, wrbuf, SEM_WR)
    cp_c = cp(c_hbm, cbuf, SEM_C)
    cp_wm = cp(wm_hbm, wmbuf, SEM_WM)
    cp_wg = cp(wg_hbm, wgbuf, SEM_WG)
    cp_wu = cp(wu_hbm, wubuf, SEM_WU)
    cp_wda = cp(wd_hbm.at[pl.ds(0, WDCUT), :], wdbuf.at[pl.ds(0, WDCUT), :], SEM_WD)
    cp_wdb = cp(wd_hbm.at[pl.ds(WDCUT, F - WDCUT), :],
                wdbuf.at[pl.ds(WDCUT, F - WDCUT), :], SEM_WD + 1)

    cp_ssm(0).start()
    cp_dd.start()
    cp_sk.start()
    for j in range(1, NJ):
        cp_ssm(j).start()
    cp_wr.start()
    cp_c.start()
    kbuf[pl.ds(0, 16), :] = jnp.zeros((16, D), BF16)
    for a in range(NA):
        cp_k(a).start()
        cp_v(a).start()
    cp_wm.start()
    for h in range(3):
        cp_q(h).start()
    cp_wg.start()
    cp_wu.start()
    cp_wda.start()
    cp_wdb.start()

    for hb in range(2):
        rho = lax.broadcasted_iota(I32, (128, 128), 0) + 128 * hb
        col = lax.broadcasted_iota(I32, (128, 128), 1)
        n8 = ((rho >> 4) << 3) + (rho & 7)
        odd = 4 * n8 + (1 if hb == 0 else -253)
        n0 = odd * (4 * col) + ((rho >> 3) & 1) * 512
        for p in range(NP):
            tab = _cos_table((n0 + p * odd) & 2047)
            gf[p, pl.ds(64 * hb, 64), :] = _pack(tab)
            gi[p, hb] = _pack(tab.T * (2.0 / 1024.0))

    cp_sk.wait()
    cp_dd.wait()
    skf = skbuf[...].astype(F32)
    ddf = ddbuf[...].astype(F32).reshape(1, D)
    for j in range(NJ):
        for m in range(4):
            prm[j, m] = jnp.broadcast_to(skf[m:m + 1, j * 128:(j + 1) * 128], (8, 128))
        prm[j, 4] = jnp.broadcast_to(ddf[:, j * 128:(j + 1) * 128], (8, 128))

    def fft4(ys, g):
        x = [(y[16 * g:16 * g + 8, :], y[16 * g + 8:16 * g + 16, :]) for y in ys]
        e0, e1 = _cadd(x[0], x[2]), _cadd(x[1], x[3])
        d0, d1 = _csub(x[0], x[2]), _csub(x[1], x[3])
        return (_cadd(e0, e1), _csub_i(d0, d1), _csub(e0, e1), _cadd_i(d0, d1))

    def cst(ref, idx, g, val):
        ref[idx + (pl.ds(16 * g, 8), slice(None))] = val[0]
        ref[idx + (pl.ds(16 * g + 8, 8), slice(None))] = val[1]

    def cld(ref, idx, g):
        return (ref[idx + (pl.ds(16 * g, 8), slice(None))],
                ref[idx + (pl.ds(16 * g + 8, 8), slice(None))])

    def fwd_k(j, carry):
        cp_ssm(j).wait()
        for a in range(NA):
            ktb[pl.ds(CH * a, CH), :] = sbuf[j, :, pl.ds(CH * a, CH)].astype(F32).T
            ys = []
            for p in range(NP):
                kp = ktb[pl.ds(CH * a + p, 128, stride=4), :].astype(BF16)
                ys.append(jnp.dot(_unpack(gf[p]), kp, preferred_element_type=F32))
            for g in range(16):
                outs = fft4(ys, g)
                for f in range(4):
                    val = outs[f]
                    if a == 0:
                        val = (val[0] + prm[j, 4], val[1])
                    if 0 < a < NA - 1:
                        cst(kraw, (a - 1, f), g, val)
                    if a > 0:
                        prev = cld(s1k, (j, f), g) if a == 1 else cld(kraw, (a - 2, f), g)
                        val = _cadd_i(val, prev) if g < 8 else _csub_i(val, prev)
                    cst(s1k, (j, 4 * a + f), g, val)
        return carry

    lax.fori_loop(0, NJ, fwd_k, 0)

    def fwd_u(a, carry):
        cp_k(a).wait()
        cp_v(a).wait()
        kc = kbuf.at[pl.ds(_mo(a * CH, CH), CH + 16)]
        vc = vbuf.at[pl.ds(_mo(a * CH, CH), CH)]
        for j in range(NJ):
            for r in range(CH // 8 + 1):
                kf[j, pl.ds(8 * r, 8), :] = kc[pl.ds(8 + 8 * r, 8), _lanes(j)].astype(F32)
            for r in range(CH // 8):
                vf[j, pl.ds(8 * r, 8), :] = vc[pl.ds(8 * r, 8), _lanes(j)].astype(F32)
            ub = [[] for _ in range(NP)]
            for b in range(16):
                seq = [kf[j, pl.ds(32 * b + 5 + m, 8, stride=4), :] for m in range(7)]
                for p in range(NP):
                    ks = ((seq[p] * prm[j, 3] + seq[p + 1] * prm[j, 2])
                          + (seq[p + 2] * prm[j, 1] + seq[p + 3] * prm[j, 0]))
                    ub[p].append(ks * vf[j, pl.ds(32 * b + p, 8, stride=4), :])
            ys = [jnp.dot(_unpack(gf[p]), jnp.concatenate(ub[p], axis=0).astype(BF16),
                          preferred_element_type=F32) for p in range(NP)]
            for g in range(16):
                outs = fft4(ys, g)
                for f in range(4):
                    cst(s1u, (j, 4 * a + f), g, outs[f])
        return carry

    lax.fori_loop(0, NA, fwd_u, 0)

    def vpu_group(j, z_ref, g):
        for a in range(NA):
            zf = []
            for f in range(4):
                acc = None
                for jj in range(a + 1):
                    t = _cmul(cld(s1u, (j, 4 * (a - jj) + f), g), cld(s1k, (j, 4 * jj + f), g))
                    acc = t if acc is None else _cadd(acc, t)
                zf.append(acc)
            e0, e1 = _cadd(zf[0], zf[2]), _csub(zf[0], zf[2])
            o0, o1 = _cadd(zf[1], zf[3]), _csub(zf[1], zf[3])
            z = (_cadd(e0, o0), _cadd_i(e1, o1), _csub(e0, o0), _csub_i(e1, o1))
            for p in range(NP):
                cst(z_ref, (4 * a + p,), g, z[p])

    def inv_unit(j, z_ref, n):
        a, p = n // NP, n % NP
        lhs = jnp.concatenate([_unpack(gi[p, 0]), _unpack(gi[p, 1])], axis=1)
        ybuf[j, pl.ds(CH * a + p, 128, stride=4), :] = jnp.dot(
            lhs, z_ref[n].astype(BF16), preferred_element_type=F32)

    for g in range(16):
        vpu_group(0, za, g)

    def v_step(i, carry):
        j = 2 * i + 1
        for g in range(16):
            inv_unit(j - 1, za, g)
            vpu_group(j, zb, g)
        for g in range(16):
            inv_unit(j, zb, g)
            vpu_group(j + 1, za, g)
        return carry

    lax.fori_loop(0, (NJ - 1) // 2, v_step, 0)

    cp_c.wait()
    cp_wr.wait()
    cp_wm.wait()
    cp_q(0).wait()
    for n in range(16):
        inv_unit(NJ - 1, za, n)
    cf = cbuf[...].astype(F32)
    sc = (cf * _sigmoid(cf)).astype(BF16)
    mod = jnp.dot(jnp.broadcast_to(sc, (16, D)), wmbuf[...],
                  preferred_element_type=F32)[0:8, :]
    mod = _rb(mod)
    sa, ca, ga, sb, cb, gb = [mod[:, i * D:(i + 1) * D] for i in range(6)]
    ca1 = _rb(1.0 + ca)
    cb1 = _rb(1.0 + cb)
    wrf = jnp.broadcast_to(wrbuf[...].astype(F32).reshape(1, D), (8, D))
    r0 = jnp.sum(wrf * sb, axis=-1, keepdims=True)
    sqd = math.sqrt(D)
    for i, val in enumerate((ga * ca1 * sqd, ga * sa, gb * cb1 * sqd, gb * sb,
                             wrf * cb1 * sqd, cb1 * sqd, sb, gb)):
        mp[i] = val

    def mrow(i):
        return [mp[i, :, _lanes(j)] for j in range(NJ)]

    lane = lax.broadcasted_iota(I32, (8, 128), 1)

    def rsum(xs):
        return jnp.broadcast_to(jnp.sum(_sum5(xs), axis=-1, keepdims=True), (8, 128))

    def brows(blk):
        return pl.ds(_mo(blk * EB * 8, EB * 8), EB * 8)

    def qtile(blk, i):
        qb = qbuf.at[brows(blk)]
        return [qb[pl.ds(8 * i, 8), _lanes(j)].astype(F32) for j in range(NJ)]

    def mix(xc, rs, y, a1, a0):
        return xc + ((xc * rs) * a1 + a0) * y

    def st1(blk, par, racc):
        for i in range(EB):
            st_m1[blk * EB + i] = rsum(qtile(blk, i)) * (1.0 / D)
        return racc

    def st2(blk, par, racc):
        for i in range(EB):
            m1 = st_m1[blk * EB + i]
            xc = [x - m1 for x in qtile(blk, i)]
            for j in range(NJ):
                ring[0, par, i, j] = xc[j]
            st_r1[blk * EB + i] = lax.rsqrt(rsum([c * c for c in xc]) + D * EPS)
        return racc

    def st3(blk, par, racc):
        a1, a0 = mrow(0), mrow(1)
        for i in range(EB):
            rs = st_r1[blk * EB + i]
            x1 = []
            for j in range(NJ):
                y = ybuf.at[j, brows(blk)][pl.ds(8 * i, 8), :]
                x1.append(mix(ring[0, par, i, j], rs, y, a1[j], a0[j]))
                ring[1, par, i, j] = x1[j]
            st_m2[blk * EB + i] = rsum(x1) * (1.0 / D)
        return racc

    def st4(blk, par, racc):
        w1 = mrow(4)
        for i in range(EB):
            m2 = st_m2[blk * EB + i]
            xc = [ring[1, par, i, j] - m2 for j in range(NJ)]
            for j in range(NJ):
                ring[2, par, i, j] = xc[j]
            rs = lax.rsqrt(rsum([c * c for c in xc]) + D * EPS)
            st_r2[blk * EB + i] = rs
            r = rsum([xc[j] * w1[j] for j in range(NJ)]) * rs
            racc = jnp.where(lane == ((blk * EB + i) & 127), r, racc)
        return racc

    def st5(blk, par, racc):
        b1, b0 = mrow(2), mrow(3)
        for i in range(EB):
            rs = st_r2[blk * EB + i]
            mm = st_m1[blk * EB + i] + st_m2[blk * EB + i]
            for j in range(NJ):
                obuf.at[brows(blk)][pl.ds(8 * i, 8), _lanes(j)] = (
                    ring[2, par, i, j] * (rs * b1[j] + 1.0) + (b0[j] + mm)).astype(BF16)
        return racc

    stages = (st1, st2, st3, st4, st5)

    def epi(n, par, racc):
        for k in reversed(range(len(stages))):
            if isinstance(n, int) and not 0 <= n - k < NB:
                continue
            racc = stages[k](n - k, (par + k) & 1, racc)
        return racc

    def epi2(i, racc):
        return epi(2 * i + 2, 0, epi(2 * i + 1, 1, racc))

    ra = jnp.zeros((8, 128), F32)
    for n in range(QFIRST):
        ra = epi(n, n & 1, ra)
    cp_q(1).wait()
    ra = lax.fori_loop(QFIRST // 2, QSPLIT // 2, epi2, ra)
    cp_q(2).wait()
    rb = lax.fori_loop(QSPLIT // 2, NB // 2 - 1, epi2, jnp.zeros((8, 128), F32))
    for n in range(NB - 1, NB + 4):
        rb = epi(n, n & 1, rb)

    bits = lax.bitcast_convert_type(_rb(jnp.concatenate([ra, rb], axis=1) + r0), I32)
    tok = (lax.broadcasted_iota(I32, (8, 256), 1) * 8
           + lax.broadcasted_iota(I32, (8, 256), 0))
    flip = lambda x: x ^ ((x >> 31) & 0x7FFF0000)
    key = flip(bits) | (S - 1 - tok)

    def amax(x):
        x = jnp.maximum(x[:, :128], x[:, 128:])
        return jnp.max(jnp.max(x, axis=0, keepdims=True), axis=1, keepdims=True)

    k1 = amax(key)
    k2 = amax(jnp.where(key == k1, jnp.iinfo(jnp.int32).min, key))
    t1 = jnp.clip(S - 1 - (k1[0, 0] & 0xFFFF), 0, S - 1)
    t2 = jnp.clip(S - 1 - (k2[0, 0] & 0xFFFF), 0, S - 1)
    m1, m2 = [lax.bitcast_convert_type(flip(kk & -65536), F32) for kk in (k1, k2)]
    c1 = t1 // (S // OCH)
    c2 = t2 // (S // OCH)

    first = lax.broadcasted_iota(I32, (8, 128), 0) == 0

    def pick(get):
        return jnp.where(first, jnp.broadcast_to(get(t1), (8, 128)),
                         jnp.broadcast_to(get(t2), (8, 128)))

    def pick_st(ref):
        return pick(lambda t: ref[t >> 3, pl.ds(t & 7, 1), :])

    rowi = lax.broadcasted_iota(I32, (16, D), 0)

    def blk16(t):
        return pl.ds(pl.multiple_of((t >> 4) << 4, 16), 16)

    def qrow(t):
        return jnp.sum(jnp.where(rowi == (t & 15), qbuf[blk16(t), :].astype(F32), 0.0),
                       axis=0, keepdims=True)

    q1, q2 = qrow(t1), qrow(t2)
    m1s, m2s, rs1, rs2 = pick_st(st_m1), pick_st(st_m2), pick_st(st_r1), pick_st(st_r2)
    a1, a0 = mrow(0), mrow(1)
    xc2 = []
    for j in range(NJ):
        xq = jnp.where(first, jnp.broadcast_to(q1[:, j * 128:(j + 1) * 128], (8, 128)),
                       jnp.broadcast_to(q2[:, j * 128:(j + 1) * 128], (8, 128)))
        y = pick(lambda t: ybuf[j, pl.ds(t, 1), :])
        xc2.append(mix(xq - m1s, rs1, y, a1[j], a0[j]) - m2s)
    mm = m1s + m2s
    cb1r, sbr, gbr = mrow(5), mrow(6), mrow(7)
    h2 = [_rb((xc2[j] * rs2) * cb1r[j] + sbr[j]) for j in range(NJ)]
    hb = jnp.concatenate(h2, axis=1).astype(BF16)
    nt = (((1,), (1,)), ((), ()))
    cp_wg.wait()
    gg = _rb(lax.dot_general(hb, wgbuf[...], nt, preferred_element_type=F32))
    gg = _rb(gg * _sigmoid(gg))
    cp_wda.wait()
    for c in range(OCH):
        @pl.when(jnp.logical_and(c1 != c, c2 != c))
        def _():
            cp_out(c).start(priority=c % 2)
    cp_wu.wait()
    uu = _rb(lax.dot_general(hb, wubuf[...], nt, preferred_element_type=F32))
    act = (gg * uu).astype(BF16)
    cp_wdb.wait()
    yy = _rb(jnp.dot(act, wdbuf[...], preferred_element_type=F32))
    yy = _rb(yy * _sigmoid(jnp.where(first[:, 0:1], m1, m2)))
    new = jnp.concatenate(
        [(xc2[j] + mm) + gbr[j] * (h2[j] + yy[:, j * 128:(j + 1) * 128]) for j in range(NJ)],
        axis=1)
    for (t, r) in ((t1, 0), (t2, 1)):
        blk = blk16(t)
        obuf[blk, :] = jnp.where(rowi == (t & 15),
                                 jnp.broadcast_to(new[r:r + 1, :], (16, D)),
                                 obuf[blk, :].astype(F32)).astype(BF16)
    cp_out(c1).start()

    @pl.when(c2 != c1)
    def _():
        cp_out(c2).start()

    for c in range(OCH):
        cp_out(c).wait()


@jax.jit
def pallas_adaLN_cond__ssm_conv_h3__moe_arch_mod__prompt_kernel(
    A_q: jax.Array,
    A_k: jax.Array,
    A_v: jax.Array,
    A_shift_k: jax.Array,
    A_ssm_k: jax.Array,
    A_ssm_D: jax.Array,
    B_x: jax.Array,
    B_w_r: jax.Array,
    B_w_gate: jax.Array,
    B_w_up: jax.Array,
    B_w_down: jax.Array,
    c: jax.Array,
    w_mod: jax.Array,
):
    del B_x
    args = (A_q, A_k, A_v, A_shift_k.T, A_ssm_k, A_ssm_D, B_w_r,
            B_w_gate.T, B_w_up.T, B_w_down, c, w_mod)
    V = pltpu.VMEM
    scratch = [
        V((S + 16, D), BF16),
        V((S, D), BF16),
        V((S, D), BF16),
        V((NJ, 128, S), BF16),
        V((D, 6 * D), BF16),
        V((F, D), BF16),
        V((F, D), BF16),
        V((F, D), BF16),
        V((4, D), BF16),
        V((D,), BF16),
        V((D,), BF16),
        V((1, D), BF16),
        V((NJ, 5, 8, 128), F32),
        V((NP, 128, 128), U32),
        V((NP, 2, 64, 128), U32),
        V((S + 8, 128), F32),
        V((NJ, CH + 16, 128), F32),
        V((NJ, CH + 8, 128), F32),
        V((NJ, 16, 256, 128), F32),
        V((NJ, 16, 256, 128), F32),
        V((2, 4, 256, 128), F32),
        V((16, 256, 128), F32),
        V((16, 256, 128), F32),
        V((NJ, S + 8, 128), F32),
        V((3, 2, EB, NJ, 8, 128), F32),
        V((S // 8, 8, 128), F32),
        V((S // 8, 8, 128), F32),
        V((S // 8, 8, 128), F32),
        V((S // 8, 8, 128), F32),
        V((S, D), BF16),
        V((8, 8, D), F32),
        pltpu.SemaphoreType.DMA((NSEM,)),
    ]
    return pl.pallas_call(
        _kernel,
        out_shape=jax.ShapeDtypeStruct((1, S, D), BF16),
        in_specs=[pl.BlockSpec(memory_space=pl.ANY)] * len(args),
        out_specs=pl.BlockSpec(memory_space=pl.ANY),
        scratch_shapes=scratch,
        compiler_params=pltpu.CompilerParams(vmem_limit_bytes=100 * 1024 * 1024,
                                             disable_semaphore_checks=True),
    )(*args)
```
